```python
import jax
import jax.numpy as jnp

def _softmax(x, axis=-1):
    return jax.nn.softmax(x, axis=axis)

def _gelu(x):
    return jax.nn.gelu(x, approximate=True)

def _silu(x):
    return jax.nn.silu(x)

def _sigmoid(x):
    return jax.nn.sigmoid(x)

def _layernorm(x, axis=-1, eps=1e-05):
    m = jnp.mean(x, axis=axis, keepdims=True)
    v = jnp.var(x, axis=axis, keepdims=True)
    return (x - m) / jnp.sqrt(v + eps)

def _scatter_add(tgt, idx, src, axis=0):
    return tgt.at[idx].add(src)

def _segment_sum(src, seg, n):
    return jax.ops.segment_sum(src, seg, n)

class _Rng:

    def __init__(self, key):
        self._k = key

    def _next(self):
        self._k, sub = jax.random.split(self._k)
        return sub

    def normal(self, shape):
        return jax.random.normal(self._next(), shape, dtype=jnp.bfloat16)

    def randint(self, lo, hi, shape):
        return jax.random.randint(self._next(), shape, lo, hi, dtype=jnp.int32)

    def uniform(self, shape, lo=0.0, hi=1.0):
        return jax.random.uniform(self._next(), shape, jnp.bfloat16, lo, hi)

    def permutation(self, n):
        return jax.random.permutation(self._next(), n)
kernel_name = 'parallel_sum__memory_aug_recurrent_mem_tr__moe_arch_mod__prompt'

def setup_inputs():
    _rng = _Rng(jax.random.key(int.from_bytes(__import__("os").urandom(4), "little")))
    _w = lambda a: (lambda t: t.astype(jnp.bfloat16) if jnp.issubdtype(t.dtype, jnp.floating) else t)(jnp.asarray(a))

    def _A_setup():
        B, S, Dm = (1, 2048, 1024)
        H, Dh = (32, 128)
        M, seg = (8, 32)
        seg = min(seg, S)
        S = S // seg * seg
        return {'x': _w((lambda *s: _rng.normal(s) * 0.05)(B, S, Dm)), 'mem0': _w((lambda *s: _rng.normal(s) * 0.05)(B, M, Dm)), 'Wq': _w((lambda *s: _rng.normal(s) * 0.05)(Dm, H, Dh) * Dm ** (-0.5)), 'Wk': _w((lambda *s: _rng.normal(s) * 0.05)(Dm, H, Dh) * Dm ** (-0.5)), 'Wv': _w((lambda *s: _rng.normal(s) * 0.05)(Dm, H, Dh) * Dm ** (-0.5)), 'Wo': _w((lambda *s: _rng.normal(s) * 0.05)(H, Dh, Dm) * (H * Dh) ** (-0.5)), 'seg_len': seg}
    _A_in = _A_setup()

    def _B_setup():
        B, S, D, F, C = (1, 2048, 1024, 3584, 2)
        return {'x': _w((lambda *s: _rng.normal(s) * 0.05)(B, S, D)), 'w_r': _w((lambda *s: _rng.normal(s) * 0.05)(D)), 'w_gate': _w((lambda *s: _rng.normal(s) * 0.05)(D, F)), 'w_up': _w((lambda *s: _rng.normal(s) * 0.05)(D, F)), 'w_down': _w((lambda *s: _rng.normal(s) * 0.05)(F, D))}
    _B_in = _B_setup()
    return {'A_x': _A_in['x'], 'A_mem0': _A_in['mem0'], 'A_Wq': _A_in['Wq'], 'A_Wk': _A_in['Wk'], 'A_Wv': _A_in['Wv'], 'A_Wo': _A_in['Wo'], 'A_seg_len': _A_in['seg_len'], 'B_x': _B_in['x'], 'B_w_r': _B_in['w_r'], 'B_w_gate': _B_in['w_gate'], 'B_w_up': _B_in['w_up'], 'B_w_down': _B_in['w_down']}

def reference(A_x, A_mem0, A_Wq, A_Wk, A_Wv, A_Wo, A_seg_len, B_x, B_w_r, B_w_gate, B_w_up, B_w_down):

    def _A_ref(x, mem0, Wq, Wk, Wv, Wo, seg_len):
        B, S, Dm = x.shape
        H, Dh = (Wq.shape[1], Wq.shape[2])
        M = mem0.shape[1]
        scale = Dh ** (-0.5)
        n_seg = S // seg_len
        L = M + seg_len
        idx = jnp.arange(L)
        mask = (idx[:, None] < M) | (idx[:, None] >= idx[None, :])
        mem = mem0
        outs = []
        for s in range(n_seg):
            xs = x[:, s * seg_len:(s + 1) * seg_len, :].copy()
            h = jnp.concatenate([mem, xs], axis=1)
            q = jnp.einsum('btd,dhe->bhte', h, Wq)
            k = jnp.einsum('btd,dhe->bhte', h, Wk)
            v = jnp.einsum('btd,dhe->bhte', h, Wv)
            scores = jnp.einsum('bhqe,bhke->bhqk', q, k) * scale
            scores = jnp.where(mask[None, None], scores, -1000000000.0)
            p = _softmax(scores, axis=-1)
            o = jnp.einsum('bhqk,bhke->bhqe', p, v)
            o = jnp.einsum('bhte,hed->btd', o, Wo)
            mem = o[:, :M, :].copy()
            outs.append(o[:, M:, :])
        return jnp.concatenate(outs, axis=1)

    def _B_ref(x, w_r, w_gate, w_up, w_down):
        B, S, D = x.shape
        C = 2
        r = x @ w_r
        idx = jnp.argsort(-r, axis=-1)[:, :C]
        idx_e = jnp.repeat(idx.reshape(B, C, 1), D, axis=2)
        x_sel = jnp.take_along_axis(x, idx_e, axis=1)
        g = _silu(x_sel @ w_gate)
        u = x_sel @ w_up
        y = g * u @ w_down
        r_sel = _sigmoid(jnp.take_along_axis(r, idx, axis=1))
        y = y * r_sel.reshape(B, C, 1)
        b_off = (jnp.arange(B) * S).reshape(B, 1)
        flat_idx = (idx + b_off).reshape(B * C)
        zero = (x * 0.0).reshape(B * S, D)
        upd = _scatter_add(zero, flat_idx, y.reshape(B * C, D), axis=0)
        return x + upd.reshape(B, S, D)
    x = A_x
    xn = _layernorm(x, axis=-1)
    return x + _A_ref(xn, A_mem0, A_Wq, A_Wk, A_Wv, A_Wo, A_seg_len) + _B_ref(xn, B_w_r, B_w_gate, B_w_up, B_w_down)
```

```python
import functools
import math

import jax
import jax.numpy as jnp
import ml_dtypes
import numpy as np
from jax import lax
from jax.experimental import pallas as pl
from jax.experimental.pallas import tpu as pltpu

F32, BF16, U32, I32 = jnp.float32, jnp.bfloat16, jnp.uint32, jnp.int32
LANES = 128
LN_EPS = float(np.asarray(1e-5, ml_dtypes.bfloat16))
MASK_VALUE = -1000000000.0
PASS_ROWS = 32
HEAD_GROUP = 2
WO_SPLITS = (16, 24)
LN_BLOCK = 64


def _round_bf16(v):
    return v.astype(BF16).astype(F32)


def _kernel(x_hbm, mem0_ref, wq_hbm, wk_hbm, wv_hbm, wo_hbm, wr_ref, wg_hbm, wu_hbm, wd_hbm,
            out_hbm,
            x_scr, xn_scr, xn0_scr, out_scr, wq_scr, wk_scr, wv_scr, wo_scr,
            stq_scr, stk_scr, stv_scr, wg_scr, wu_scr, wd_scr,
            mem_scr, o_scr, acc_scr, top_scr, topi_scr, sems, *rings,
            S, D, H, E, M, SEG, FF, TP, T0, RING, RING_OFF):
    L = M + SEG
    n_seg = S // SEG
    KT = D // LANES
    chunk_rows = LANES * H
    piece = (S - T0) // KT
    w_hbm = (wq_hbm, wk_hbm, wv_hbm)
    w_scr = (wq_scr, wk_scr, wv_scr)
    st_scr = (stq_scr, stk_scr, stv_scr)
    SEM_X, SEM_W, SEM_WO, SEM_FFN, SEM_OUT, SEM_FIX = 0, 1, 4, 5, 6, 7

    def x_copy(start, rows):
        return pltpu.make_async_copy(
            x_hbm.at[pl.ds(start, rows)], x_scr.at[pl.ds(start, rows)], sems.at[SEM_X])

    def x_piece_copy(i):
        return x_copy(pl.multiple_of(T0 + i * piece, 16), piece)

    def w_copy(m, i):
        start = i * chunk_rows
        if not isinstance(start, int):
            start = pl.multiple_of(start, chunk_rows)
        return pltpu.make_async_copy(
            w_hbm[m].at[pl.ds(start, chunk_rows)], st_scr[m], sems.at[SEM_W + m])

    def column_copy(src, dst, j, sem):
        start = j * LANES
        if not isinstance(start, int):
            start = pl.multiple_of(start, LANES)
        return pltpu.make_async_copy(src.at[:, pl.ds(start, LANES)], dst.at[j], sems.at[sem])

    ffn_copies = (
        [column_copy(wg_hbm, wg_scr, j, SEM_FFN) for j in range(FF // LANES)]
        + [column_copy(wu_hbm, wu_scr, j, SEM_FFN) for j in range(FF // LANES)]
        + [column_copy(wd_hbm, wd_scr, j, SEM_FFN) for j in range(KT)])

    def load_packed(ref, *idx):
        return pltpu.bitcast(ref[idx], BF16)

    def layernorm(xb):
        mean = jnp.sum(xb, axis=-1, keepdims=True) * (1.0 / D)
        cen = xb - mean
        var = jnp.sum(cen * cen, axis=-1, keepdims=True) * (1.0 / D)
        std = _round_bf16(jnp.sqrt(_round_bf16(_round_bf16(var) + LN_EPS)))
        return _round_bf16(_round_bf16(xb - _round_bf16(mean)) / std)

    def normalise_rows(start, prologue_rows):
        xn = layernorm(x_scr[pl.ds(start, LN_BLOCK), :].astype(F32))
        xn_scr[pl.ds(start, LN_BLOCK), :] = xn
        if prologue_rows:
            for j in range(KT):
                xn0_scr[j, pl.ds(start, LN_BLOCK), :] = xn[:, j * LANES:(j + 1) * LANES].astype(BF16)
        score = _round_bf16(jnp.sum(xn * wr_ref[...].astype(F32), axis=-1, keepdims=True))
        best1, best2, idx1, idx2 = top_scr[0], top_scr[1], topi_scr[0], topi_scr[1]
        sub = lax.broadcasted_iota(I32, (8, LANES), 0)
        for b in range(LN_BLOCK // 8):
            r = jnp.broadcast_to(score[8 * b:8 * b + 8], (8, LANES))
            row = sub + (start + 8 * b)
            gt1, gt2 = r > best1, r > best2
            best2 = jnp.where(gt1, best1, jnp.where(gt2, r, best2))
            idx2 = jnp.where(gt1, idx1, jnp.where(gt2, row, idx2))
            best1 = jnp.where(gt1, r, best1)
            idx1 = jnp.where(gt1, row, idx1)
        top_scr[0], top_scr[1], topi_scr[0], topi_scr[1] = best1, best2, idx1, idx2

    def relayout(m, i):
        src = st_scr[m].bitcast(U32)
        hp = H // 2
        for g in range(LANES // 16):
            w = src[g * 16 * hp:(g + 1) * 16 * hp, :].reshape(8, 2, hp, E)
            lo, hi = w[:, 0], w[:, 1]
            even = (lo & 0xFFFF) | (hi << 16)
            odd = (lo >> 16) | (hi & np.uint32(0xFFFF0000))
            rows = pl.ds(pl.multiple_of(i * (LANES // 2) + g * 8, 8), 8)
            for b in range(hp // 8):
                even_t = jnp.swapaxes(even[:, 8 * b:8 * b + 8, :], 0, 1)
                odd_t = jnp.swapaxes(odd[:, 8 * b:8 * b + 8, :], 0, 1)
                for j in range(8):
                    w_scr[m][2 * (8 * b + j), rows, :] = even_t[j]
                    w_scr[m][2 * (8 * b + j) + 1, rows, :] = odd_t[j]

    def project_first_tokens(m, i):
        rows = pl.ds(pl.multiple_of(i * (LANES // 2), LANES // 2), LANES // 2)
        for h0 in range(0, H, 4):
            w = jnp.concatenate([load_packed(w_scr[m], h0 + t, rows) for t in range(4)], axis=1)
            r = jnp.dot(xn0_scr[i], w, preferred_element_type=F32)
            for t in range(4):
                old = rings[h0 + t][m, RING_OFF:RING_OFF + T0, :]
                rings[h0 + t][m, RING_OFF:RING_OFF + T0, :] = (
                    r[:, t * E:(t + 1) * E] + jnp.where(i > 0, old, 0.0))

    x_copy(0, T0 + piece).start()
    w_copy(0, 0).start()
    w_copy(1, 0).start()
    mem_scr[...] = mem0_ref[...].astype(F32)
    top_scr[...] = jnp.full(top_scr.shape, -jnp.inf, F32)
    topi_scr[0] = lax.broadcasted_iota(I32, (8, LANES), 0)
    topi_scr[1] = lax.broadcasted_iota(I32, (8, LANES), 0) + 8
    x_copy(0, T0 + piece).wait()
    w_copy(2, 0).start()

    @pl.loop(0, T0 // LN_BLOCK)
    def _(b):
        normalise_rows(pl.multiple_of(b * LN_BLOCK, LN_BLOCK), True)

    w_copy(0, 0).wait()
    relayout(0, 0)

    @pl.loop(0, KT)
    def _(i):
        more = i + 1 < KT

        @pl.when(i > 0)
        def _():
            x_piece_copy(i).wait()

        for m in range(3):
            if m < 2:
                w_copy(m + 1, i).wait()

            @pl.when(more)
            def _():
                if m == 2:
                    w_copy(0, i + 1).wait()
                w_copy(m, i + 1).start()
                if m == 0:
                    x_piece_copy(i + 1).start()

            if m == 1:
                column_copy(wo_hbm, wo_scr, i, SEM_WO).start()
            project_first_tokens(m, i)
            if m < 2:
                relayout(m + 1, i)
            else:
                relayout(0, jnp.minimum(i + 1, KT - 1))
            for b in range(piece // (3 * LN_BLOCK)):
                start = T0 + i * piece + (m * (piece // 3) + b * LN_BLOCK)
                normalise_rows(pl.multiple_of(start, LN_BLOCK), False)

    for j in range(KT):
        column_copy(wo_hbm, wo_scr, j, SEM_WO).wait()
    for c in ffn_copies:
        c.start()

    wo_words = wo_scr.bitcast(U32)
    scale = E ** -0.5

    @pl.loop(0, n_seg)
    def _(s):
        q_row = lax.broadcasted_iota(I32, (L, L), 0)
        k_col = lax.broadcasted_iota(I32, (L, L), 1)
        visible = (q_row < M) | (q_row >= k_col)
        seg_rows = pl.ds(pl.multiple_of(s * SEG, SEG), SEG)
        new_rows = pl.ds(pl.multiple_of(T0 + s * TP, 8), TP)
        put = pl.ds(pl.multiple_of(lax.rem(RING_OFF + T0 + s * TP, RING), 8), TP)
        get = pl.ds(pl.multiple_of(lax.rem(RING_OFF + s * SEG, RING), 8), SEG)
        mem_qkv, probs = {}, {}

        def project(g):
            lhs = jnp.concatenate([mem_scr[...], xn_scr[new_rows, :]], axis=0)
            for h in range(g * HEAD_GROUP, (g + 1) * HEAD_GROUP):
                w = jnp.concatenate([load_packed(w_scr[m], h) for m in range(3)], axis=1)
                r = jnp.dot(lhs, w, preferred_element_type=F32)
                mem_qkv[h] = [r[:M, m * E:(m + 1) * E] for m in range(3)]
                for m in range(3):
                    rings[h][m, put, :] = r[M:, m * E:(m + 1) * E]

        def segment(h, m):
            return jnp.concatenate([mem_qkv[h][m], rings[h][m, get, :]], axis=0)

        def attend(g):
            for h in range(g * HEAD_GROUP, (g + 1) * HEAD_GROUP):
                sc = lax.dot_general(segment(h, 0), segment(h, 1).astype(BF16),
                                     (((1,), (1,)), ((), ())), preferred_element_type=F32)
                sc = jnp.where(visible, sc * scale, MASK_VALUE)
                e = jnp.exp(sc - jnp.max(sc, axis=-1, keepdims=True))
                probs[h] = e / jnp.sum(e, axis=-1, keepdims=True)

        def mix(g):
            for h in range(g * HEAD_GROUP, (g + 1) * HEAD_GROUP):
                o_scr[:, h * E:(h + 1) * E] = jnp.dot(
                    probs[h], segment(h, 2).astype(BF16), preferred_element_type=F32)

        def output(h0, h1):
            o = o_scr[:, h0 * E:h1 * E]
            for j in range(KT):
                cols = slice(j * LANES, (j + 1) * LANES)
                r = jnp.dot(o, load_packed(wo_words, j, slice(h0 * E // 2, h1 * E // 2)),
                            preferred_element_type=F32)
                if h0 > 0:
                    r = r + acc_scr[:, cols]
                if h1 < H:
                    acc_scr[:, cols] = r
                else:
                    mem_scr[:, cols] = r[:M]
                    total = x_scr[seg_rows, cols].astype(F32) + r[M:] + xn_scr[seg_rows, cols]
                    out_scr[seg_rows, cols] = total.astype(out_scr.dtype)

        n_groups = H // HEAD_GROUP
        bounds = (0,) + WO_SPLITS + (H,)
        done = 0
        for t in range(n_groups + 2):
            if t < n_groups:
                project(t)
            elif done < len(bounds) - 2:
                output(bounds[done], bounds[done + 1])
                done += 1
            if 0 <= t - 1 < n_groups:
                attend(t - 1)
            if 0 <= t - 2 < n_groups:
                mix(t - 2)
        for d in range(done, len(bounds) - 1):
            output(bounds[d], bounds[d + 1])
        pltpu.make_async_copy(out_scr.at[seg_rows], out_hbm.at[seg_rows], sems.at[SEM_OUT]).start()

    best1, best2, idx1, idx2 = top_scr[0], top_scr[1], topi_scr[0], topi_scr[1]
    r_a = jnp.max(best1, axis=0, keepdims=True)
    i_a = jnp.min(jnp.where(best1 == r_a, idx1, S - 1), axis=0, keepdims=True)
    rest = jnp.where(idx1 == i_a, best2, best1)
    rest_idx = jnp.where(idx1 == i_a, idx2, idx1)
    r_b = jnp.max(rest, axis=0, keepdims=True)
    i_b = jnp.min(jnp.where((rest == r_b) & (rest_idx != i_a), rest_idx, S - 1),
                  axis=0, keepdims=True)
    rows = [jnp.clip(jnp.max(i), 0, S - 1) for i in (i_a, i_b)]

    sub = lax.broadcasted_iota(I32, (8, D), 0)
    x_sel = jnp.where(sub == 0, xn_scr[pl.ds(rows[0], 1), :],
                      jnp.where(sub == 1, xn_scr[pl.ds(rows[1], 1), :], 0.0))
    for c in ffn_copies:
        c.wait()
    wg_words, wu_words, wd_words = (r.bitcast(U32) for r in (wg_scr, wu_scr, wd_scr))
    hidden = []
    for j in range(FF // LANES):
        w = jnp.concatenate([load_packed(wg_words, j), load_packed(wu_words, j)], axis=1)
        r = jnp.dot(x_sel, w, preferred_element_type=F32)
        gate, up = r[:, :LANES], r[:, LANES:]
        hidden.append(gate * jax.nn.sigmoid(gate) * up)
    hidden = jnp.concatenate(hidden, axis=1)
    y = jnp.concatenate(
        [jnp.dot(hidden, load_packed(wd_words, j), preferred_element_type=F32) for j in range(KT)],
        axis=1)

    pltpu.make_async_copy(out_scr, out_hbm, sems.at[SEM_OUT]).wait()
    tiles = [pl.ds(pl.multiple_of(row // 16 * 16, 16), 16) for row in rows]
    for c, r_c in enumerate((r_a, r_b)):
        weight = jnp.concatenate([jax.nn.sigmoid(r_c)] * KT, axis=1)
        old = out_scr[tiles[c], :].astype(F32)
        hit = lax.broadcasted_iota(I32, (16, D), 0) == lax.rem(rows[c], 16)
        out_scr[tiles[c], :] = jnp.where(hit, old + y[c:c + 1] * weight, old).astype(out_scr.dtype)

    def fix_copy(c):
        return pltpu.make_async_copy(
            out_scr.at[tiles[c]], out_hbm.at[tiles[c]], sems.at[SEM_FIX + c])

    fix_copy(0).start()

    @pl.when(rows[0] // 16 != rows[1] // 16)
    def _():
        fix_copy(1).start()
        fix_copy(1).wait()

    fix_copy(0).wait()


@functools.partial(jax.jit, static_argnames=("A_seg_len",))
def pallas_parallel_sum__memory_aug_recurrent_mem_tr__moe_arch_mod__prompt_kernel(
    A_x, A_mem0, A_Wq, A_Wk, A_Wv, A_Wo, A_seg_len, B_x, B_w_r, B_w_gate, B_w_up, B_w_down,
):
    del B_x
    B, S, D = A_x.shape
    _, H, E = A_Wq.shape
    M, SEG, FF = A_mem0.shape[1], int(A_seg_len), B_w_gate.shape[1]
    KT = D // LANES
    TP = PASS_ROWS - M
    T0 = S - (S // SEG) * TP
    period = math.lcm(TP, SEG)
    RING = -(-(T0 + TP) // period) * period
    RING_OFF = RING - T0
    assert B == 1 and E == LANES and M == 8 and SEG % 16 == 0 and S % SEG == 0
    assert H % 16 == 0 and D % LANES == 0 and FF % LANES == 0
    assert 0 < TP <= SEG and TP % 8 == 0 and RING_OFF % SEG == 0
    assert T0 % LN_BLOCK == 0 and (S - T0) % (3 * KT * LN_BLOCK) == 0

    hbm = pl.BlockSpec(memory_space=pl.ANY)
    vmem = pl.BlockSpec(memory_space=pltpu.VMEM)
    scratch = [
        pltpu.VMEM((S, D), A_x.dtype),
        pltpu.VMEM((S, D), F32),
        pltpu.VMEM((KT, T0, LANES), BF16),
        pltpu.VMEM((S, D), A_x.dtype),
        *[pltpu.VMEM((H, D // 2, E), U32)] * 3,
        pltpu.VMEM((KT, H * E, LANES), BF16),
        *[pltpu.VMEM((LANES * H, E), BF16)] * 3,
        *[pltpu.VMEM((FF // LANES, D, LANES), BF16)] * 2,
        pltpu.VMEM((KT, FF, LANES), BF16),
        pltpu.VMEM((M, D), F32),
        pltpu.VMEM((M + SEG, H * E), F32),
        pltpu.VMEM((M + SEG, D), F32),
        pltpu.VMEM((2, 8, LANES), F32),
        pltpu.VMEM((2, 8, LANES), I32),
        pltpu.SemaphoreType.DMA((9,)),
        *[pltpu.VMEM((3, RING, E), F32)] * H,
    ]
    out = pl.pallas_call(
        functools.partial(_kernel, S=S, D=D, H=H, E=E, M=M, SEG=SEG, FF=FF, TP=TP, T0=T0,
                          RING=RING, RING_OFF=RING_OFF),
        out_shape=jax.ShapeDtypeStruct((S, D), A_x.dtype),
        in_specs=[hbm, vmem, hbm, hbm, hbm, hbm, vmem, hbm, hbm, hbm],
        out_specs=hbm,
        scratch_shapes=scratch,
        compiler_params=pltpu.CompilerParams(vmem_limit_bytes=120 * 1024 * 1024),
        name="rmt_mod",
    )(A_x.reshape(S, D), A_mem0.reshape(M, D),
      A_Wq.reshape(D * H, E), A_Wk.reshape(D * H, E), A_Wv.reshape(D * H, E),
      A_Wo.reshape(H * E, D), B_w_r.reshape(1, D), B_w_gate, B_w_up, B_w_down)
    return out.reshape(B, S, D)
```

```python
import functools
import math

import jax
import jax.numpy as jnp
import ml_dtypes
import numpy as np
from jax import lax
from jax.experimental import pallas as pl
from jax.experimental.pallas import tpu as pltpu

F32, BF16, U32, I32 = jnp.float32, jnp.bfloat16, jnp.uint32, jnp.int32
LANES = 128
LN_EPS = float(np.asarray(1e-5, ml_dtypes.bfloat16))
MASK_VALUE = -1000000000.0
PASS_ROWS = 32
PASSES_PER_STEP = 4
HEAD_GROUP = 2
SCORE_LAG, MIX_LAG = 2, 1
WO_SPLITS = (8, 16, 22, 28)
X_PARTS = 2


def _round_bf16(v):
    return v.astype(BF16).astype(F32)


def _load_packed(ref, *idx):
    return pltpu.bitcast(ref[idx], BF16)


def _paced(bits, after):
    return (pltpu.bitcast(after, U32) | bits) & bits


def _aligned(i, n):
    return i if isinstance(i, int) else pl.multiple_of(i, n)


def _kernel(x_hbm, mem0_ref, wq_hbm, wk_hbm, wv_hbm, wo_hbm, wr_ref, wg_hbm, wu_hbm, wd_hbm,
            out_hbm,
            x_scr, xn_scr, xn0_scr, out_scr, wq_scr, wk_scr, wv_scr, wo_scr,
            stq_scr, stk_scr, stv_scr, wg_scr, wu_scr, wd_scr,
            mem_scr, o_scr, acc_scr, wr_scr, top_scr, topi_scr, sems, *rings,
            S, D, H, E, M, SEG, FF, TP, T0, RING):
    L = M + SEG
    KT = D // LANES
    RING_OFF = RING - T0
    chunk_rows = LANES * H
    piece = (S - T0) // KT
    part = T0 // X_PARTS
    w_hbm = (wq_hbm, wk_hbm, wv_hbm)
    w_scr = (wq_scr, wk_scr, wv_scr)
    st_scr = (stq_scr, stk_scr, stv_scr)
    SEM_X, SEM_W, SEM_WO, SEM_FFN, SEM_OUT, SEM_FIX, SEM_PART = 0, 1, 4, 5, 6, 7, 9

    def x_copy(start, rows, sem):
        return pltpu.make_async_copy(
            x_hbm.at[pl.ds(start, rows)], x_scr.at[pl.ds(start, rows)], sems.at[sem])

    def x_piece_copy(i):
        return x_copy(_aligned(T0 + i * piece, 16), piece, SEM_X)

    def w_copy(m, i):
        return pltpu.make_async_copy(
            w_hbm[m].at[pl.ds(_aligned(i * chunk_rows, chunk_rows), chunk_rows)],
            st_scr[m], sems.at[SEM_W + m])

    def column_copy(src, dst, j, sem):
        return pltpu.make_async_copy(
            src.at[:, pl.ds(_aligned(j * LANES, LANES), LANES)], dst.at[j], sems.at[sem])

    def out_copy(start, rows, sem):
        return pltpu.make_async_copy(
            out_scr.at[pl.ds(start, rows)], out_hbm.at[pl.ds(start, rows)], sems.at[sem])

    ffn_copies = (
        [column_copy(wg_hbm, wg_scr, j, SEM_FFN) for j in range(FF // LANES)]
        + [column_copy(wu_hbm, wu_scr, j, SEM_FFN) for j in range(FF // LANES)]
        + [column_copy(wd_hbm, wd_scr, j, SEM_FFN) for j in range(KT)])

    def layernorm(xb):
        mean = jnp.sum(xb, axis=-1, keepdims=True) * (1.0 / D)
        cen = xb - mean
        var = jnp.sum(cen * cen, axis=-1, keepdims=True) * (1.0 / D)
        std = _round_bf16(jnp.sqrt(_round_bf16(_round_bf16(var) + LN_EPS)))
        return _round_bf16(_round_bf16(xb - _round_bf16(mean)) / std)

    def normalise_rows(start, rows, after=None):
        xb = x_scr[pl.ds(start, rows), :].astype(F32)
        if after is not None:
            one = pltpu.bitcast(_paced(0x3F800000, after[:rows, :LANES]), F32)
            xb = xb * jnp.concatenate([one] * KT, axis=1)
        xn = layernorm(xb)
        xn_scr[pl.ds(start, rows), :] = xn
        wr = jnp.concatenate([wr_scr[...]] * (rows // 8), axis=0)
        score = _round_bf16(jnp.sum(xn * wr, axis=-1, keepdims=True))
        best1, best2, idx1, idx2 = top_scr[0], top_scr[1], topi_scr[0], topi_scr[1]
        sub = lax.broadcasted_iota(I32, (8, LANES), 0)
        for b in range(rows // 8):
            r = jnp.broadcast_to(score[8 * b:8 * b + 8], (8, LANES))
            row = sub + (start + 8 * b)
            gt1, gt2 = r > best1, r > best2
            best2 = jnp.where(gt1, best1, jnp.where(gt2, r, best2))
            idx2 = jnp.where(gt1, idx1, jnp.where(gt2, row, idx2))
            best1 = jnp.where(gt1, r, best1)
            idx1 = jnp.where(gt1, row, idx1)
        top_scr[0], top_scr[1], topi_scr[0], topi_scr[1] = best1, best2, idx1, idx2
        return xn

    def relayout(m, i, g, after=None):
        src = st_scr[m].bitcast(U32)
        hp = H // 2
        w = src[g * 16 * hp:(g + 1) * 16 * hp, :].reshape(8, 2, hp, E)
        lo, hi = w[:, 0], w[:, 1]
        rows = pl.ds(_aligned(i * (LANES // 2) + g * 8, 8), 8)
        for b in range(hp // 8):
            heads = slice(8 * b, 8 * b + 8)
            shift = [16, 16]
            if after is not None:
                for u in range(2):
                    r0 = (2 * b + u) * (T0 // (hp // 4))
                    shift[u] = _paced(16, after[r0:r0 + 8, :LANES])[None]
            even = (lo[:, heads] & 0xFFFF) | (hi[:, heads] << shift[0])
            odd = (lo[:, heads] >> shift[1]) | (hi[:, heads] & np.uint32(0xFFFF0000))
            even, odd = jnp.swapaxes(even, 0, 1), jnp.swapaxes(odd, 0, 1)
            for j in range(8):
                w_scr[m][2 * (8 * b + j), rows, :] = even[j]
                w_scr[m][2 * (8 * b + j) + 1, rows, :] = odd[j]

    def project_first_tokens(m, i, h0):
        rows = pl.ds(_aligned(i * (LANES // 2), LANES // 2), LANES // 2)
        w = jnp.concatenate([_load_packed(w_scr[m], h0 + t, rows) for t in range(4)], axis=1)
        r = jnp.dot(_load_packed(xn0_scr, i), w, preferred_element_type=F32)
        for t in range(4):
            old = rings[h0 + t][m, RING_OFF:RING, :]
            rings[h0 + t][m, RING_OFF:RING, :] = r[:, t * E:(t + 1) * E] + jnp.where(i > 0, old, 0.0)
        return r

    for p in range(X_PARTS):
        x_copy(p * part, part, SEM_PART + p).start()
    w_copy(0, 0).start()
    w_copy(1, 0).start()
    x_piece_copy(0).start()
    w_copy(2, 0).start()
    mem_scr[...] = mem0_ref[...].astype(F32)
    wr_scr[...] = jnp.broadcast_to(wr_ref[...].astype(F32).reshape(1, D), wr_scr.shape)
    top_scr[...] = jnp.full(top_scr.shape, -jnp.inf, F32)
    topi_scr[0] = lax.broadcasted_iota(I32, (8, LANES), 0)
    topi_scr[1] = lax.broadcasted_iota(I32, (8, LANES), 0) + 8
    for p in range(X_PARTS):
        x_copy(p * part, part, SEM_PART + p).wait()
        for r0 in range(p * part, (p + 1) * part, 64):
            xn = normalise_rows(r0, 64)
            for j in range(KT):
                xn0_scr[j, r0 // 2:(r0 + 64) // 2, :] = pltpu.bitcast(
                    xn[:, j * LANES:(j + 1) * LANES].astype(BF16), U32)
    w_copy(0, 0).wait()
    for g in range(LANES // 16):
        relayout(0, 0, g)

    @pl.loop(0, KT)
    def _(i):
        for m in range(3):
            if m < 2:
                w_copy(m + 1, i).wait()
            if m == 1:
                x_piece_copy(i).wait()

            @pl.when(i + 1 < KT)
            def _():
                if m == 2:
                    w_copy(0, i + 1).wait()
                w_copy(m, i + 1).start()
                if m == 1:
                    x_piece_copy(i + 1).start()

            if m == 1:
                column_copy(wo_hbm, wo_scr, i, SEM_WO).start()
            nxt = (m + 1, i) if m < 2 else (0, jnp.minimum(i + 1, KT - 1))
            after = None
            for g in range(LANES // 16):
                relayout(*nxt, g, after)
                if m > 0 and 1 <= g <= piece // 32:
                    start = T0 + i * piece + ((m - 1) * (piece // 2) + (g - 1) * 16)
                    normalise_rows(_aligned(start, 16), 16, after)
                after = project_first_tokens(m, i, 4 * g)

    for j in range(KT):
        column_copy(wo_hbm, wo_scr, j, SEM_WO).wait()
    for c in ffn_copies:
        c.start()

    wo_words = wo_scr.bitcast(U32)
    log2e = math.log2(math.e)

    def one_pass(s):
        q_row = lax.broadcasted_iota(I32, (L, L), 0)
        k_col = lax.broadcasted_iota(I32, (L, L), 1)
        visible = (q_row < M) | (q_row >= k_col)
        seg_rows = pl.ds(_aligned(s * SEG, SEG), SEG)
        put = pl.ds(_aligned(lax.rem(RING + s * TP, RING), 8), TP)
        get = pl.ds(_aligned(lax.rem(RING_OFF + s * SEG, RING), 8), SEG)
        lhs = jnp.concatenate(
            [xn_scr[pl.ds(_aligned(T0 + s * TP, 8), TP), :], mem_scr[...]], axis=0).astype(BF16)
        mem_qkv, probs = {}, {}

        def heads(g):
            return range(g * HEAD_GROUP, (g + 1) * HEAD_GROUP)

        def project(g):
            for h in heads(g):
                w = jnp.concatenate([_load_packed(w_scr[m], h) for m in range(3)], axis=1)
                r = jnp.dot(lhs, w, preferred_element_type=F32)
                mem_qkv[h] = [r[TP:, m * E:(m + 1) * E] for m in range(3)]
                for m in range(3):
                    rings[h][m, put, :] = r[:TP, m * E:(m + 1) * E]

        def segment(h, m):
            return jnp.concatenate([mem_qkv[h][m], rings[h][m, get, :]], axis=0)

        def attend(g):
            for h in heads(g):
                sc = lax.dot_general(segment(h, 0), segment(h, 1).astype(BF16),
                                     (((1,), (1,)), ((), ())), preferred_element_type=F32)
                sc = jnp.where(visible, sc * (E ** -0.5 * log2e), MASK_VALUE * log2e)
                e = jnp.exp2(sc - jnp.max(sc, axis=-1, keepdims=True))
                probs[h] = e / jnp.sum(e, axis=-1, keepdims=True)

        def mix(g):
            for h in heads(g):
                o_scr[:, h * E:(h + 1) * E] = jnp.dot(
                    probs[h], segment(h, 2).astype(BF16), preferred_element_type=F32)

        def output(h0, h1):
            o = o_scr[:, h0 * E:h1 * E]
            for j in range(KT):
                cols = slice(j * LANES, (j + 1) * LANES)
                r = jnp.dot(o, _load_packed(wo_words, j, slice(h0 * E // 2, h1 * E // 2)),
                            preferred_element_type=F32)
                if h0 > 0:
                    r = r + acc_scr[:, cols]
                else:
                    base = x_scr[seg_rows, cols].astype(F32) + xn_scr[seg_rows, cols]
                    r = jnp.concatenate([r[:M], r[M:] + base], axis=0)
                if h1 < H:
                    acc_scr[:, cols] = r
                else:
                    mem_scr[:, cols] = r[:M]
                    out_scr[seg_rows, cols] = r[M:].astype(out_scr.dtype)

        n_groups = H // HEAD_GROUP
        bounds = (0,) + WO_SPLITS + (H,)
        done = 0
        for t in range(n_groups + SCORE_LAG + MIX_LAG):
            if t < n_groups:
                project(t)
            elif done < len(WO_SPLITS):
                assert bounds[done + 1] <= (t - SCORE_LAG - MIX_LAG) * HEAD_GROUP
                output(bounds[done], bounds[done + 1])
                done += 1
            if 0 <= t - SCORE_LAG - MIX_LAG < n_groups:
                mix(t - SCORE_LAG - MIX_LAG)
            if 0 <= t - SCORE_LAG < n_groups:
                attend(t - SCORE_LAG)
        for d in range(done, len(bounds) - 1):
            output(bounds[d], bounds[d + 1])

    step_rows = PASSES_PER_STEP * SEG

    @pl.loop(0, S // step_rows)
    def _(step):
        for u in range(PASSES_PER_STEP):
            one_pass(step * PASSES_PER_STEP + u)
        out_copy(_aligned(step * step_rows, step_rows), step_rows, SEM_OUT).start()

    best1, best2, idx1, idx2 = top_scr[0], top_scr[1], topi_scr[0], topi_scr[1]
    r_a = jnp.max(best1, axis=0, keepdims=True)
    i_a = jnp.min(jnp.where(best1 == r_a, idx1, S - 1), axis=0, keepdims=True)
    rest = jnp.where(idx1 == i_a, best2, best1)
    rest_idx = jnp.where(idx1 == i_a, idx2, idx1)
    r_b = jnp.max(rest, axis=0, keepdims=True)
    i_b = jnp.min(jnp.where((rest == r_b) & (rest_idx != i_a), rest_idx, S - 1),
                  axis=0, keepdims=True)
    picked = [jnp.clip(jnp.max(i), 0, S - 1) for i in (i_a, i_b)]

    sub = lax.broadcasted_iota(I32, (8, D), 0)
    x_sel = jnp.where(sub == 0, xn_scr[pl.ds(picked[0], 1), :],
                      jnp.where(sub == 1, xn_scr[pl.ds(picked[1], 1), :], 0.0))
    for c in ffn_copies:
        c.wait()
    wg_words, wu_words, wd_words = (r.bitcast(U32) for r in (wg_scr, wu_scr, wd_scr))
    hidden = []
    for j in range(FF // LANES):
        w = jnp.concatenate([_load_packed(wg_words, j), _load_packed(wu_words, j)], axis=1)
        r = jnp.dot(x_sel, w, preferred_element_type=F32)
        gate, up = r[:, :LANES], r[:, LANES:]
        hidden.append(gate * jax.nn.sigmoid(gate) * up)
    hidden = jnp.concatenate(hidden, axis=1)
    y = jnp.concatenate(
        [jnp.dot(hidden, _load_packed(wd_words, j), preferred_element_type=F32) for j in range(KT)],
        axis=1)

    out_copy(0, S, SEM_OUT).wait()
    tiles = [_aligned(row // 16 * 16, 16) for row in picked]
    for c, r_c in enumerate((r_a, r_b)):
        weight = jnp.concatenate([jax.nn.sigmoid(r_c)] * KT, axis=1)
        old = out_scr[pl.ds(tiles[c], 16), :].astype(F32)
        hit = lax.broadcasted_iota(I32, (16, D), 0) == lax.rem(picked[c], 16)
        out_scr[pl.ds(tiles[c], 16), :] = jnp.where(
            hit, old + y[c:c + 1] * weight, old).astype(out_scr.dtype)

    out_copy(tiles[0], 16, SEM_FIX).start()

    @pl.when(tiles[0] != tiles[1])
    def _():
        out_copy(tiles[1], 16, SEM_FIX + 1).start()
        out_copy(tiles[1], 16, SEM_FIX + 1).wait()

    out_copy(tiles[0], 16, SEM_FIX).wait()


@functools.partial(jax.jit, static_argnames=("A_seg_len",))
def pallas_parallel_sum__memory_aug_recurrent_mem_tr__moe_arch_mod__prompt_kernel(
    A_x, A_mem0, A_Wq, A_Wk, A_Wv, A_Wo, A_seg_len, B_x, B_w_r, B_w_gate, B_w_up, B_w_down,
):
    del B_x
    B, S, D = A_x.shape
    _, H, E = A_Wq.shape
    M, SEG, FF = A_mem0.shape[1], int(A_seg_len), B_w_gate.shape[1]
    KT = D // LANES
    TP = PASS_ROWS - M
    T0 = S - (S // SEG) * TP
    period = math.lcm(TP, SEG)
    RING = -(-(T0 + TP) // period) * period
    assert B == 1 and E == LANES and M == 8 and H == 32 and D % LANES == 0 and FF % LANES == 0
    assert SEG % 16 == 0 and S % (SEG * PASSES_PER_STEP) == 0 and 0 < TP <= SEG and TP % 8 == 0
    assert (RING - T0) % SEG == 0 and T0 % (64 * X_PARTS) == 0
    assert (S - T0) % (32 * KT) == 0 and (S - T0) // (32 * KT) < LANES // 16

    hbm = pl.BlockSpec(memory_space=pl.ANY)
    vmem = pl.BlockSpec(memory_space=pltpu.VMEM)
    scratch = [
        pltpu.VMEM((S, D), A_x.dtype),
        pltpu.VMEM((S, D), F32),
        pltpu.VMEM((KT, T0 // 2, LANES), U32),
        pltpu.VMEM((S, D), A_x.dtype),
        *[pltpu.VMEM((H, D // 2, E), U32)] * 3,
        pltpu.VMEM((KT, H * E, LANES), BF16),
        *[pltpu.VMEM((LANES * H, E), BF16)] * 3,
        *[pltpu.VMEM((FF // LANES, D, LANES), BF16)] * 2,
        pltpu.VMEM((KT, FF, LANES), BF16),
        pltpu.VMEM((M, D), F32),
        pltpu.VMEM((M + SEG, H * E), F32),
        pltpu.VMEM((M + SEG, D), F32),
        pltpu.VMEM((8, D), F32),
        pltpu.VMEM((2, 8, LANES), F32),
        pltpu.VMEM((2, 8, LANES), I32),
        pltpu.SemaphoreType.DMA((9 + X_PARTS,)),
        *[pltpu.VMEM((3, RING, E), F32)] * H,
    ]
    out = pl.pallas_call(
        functools.partial(_kernel, S=S, D=D, H=H, E=E, M=M, SEG=SEG, FF=FF, TP=TP, T0=T0, RING=RING),
        out_shape=jax.ShapeDtypeStruct((S, D), A_x.dtype),
        in_specs=[hbm, vmem, hbm, hbm, hbm, hbm, vmem, hbm, hbm, hbm],
        out_specs=hbm,
        scratch_shapes=scratch,
        compiler_params=pltpu.CompilerParams(
            vmem_limit_bytes=120 * 1024 * 1024, disable_bounds_checks=True),
        name="rmt_mod",
    )(A_x.reshape(S, D), A_mem0.reshape(M, D),
      A_Wq.reshape(D * H, E), A_Wk.reshape(D * H, E), A_Wv.reshape(D * H, E),
      A_Wo.reshape(H * E, D), B_w_r, B_w_gate, B_w_up, B_w_down)
    return out.reshape(B, S, D)
```

```python
import functools
import math

import jax
import jax.numpy as jnp
import ml_dtypes
import numpy as np
from jax import lax
from jax.experimental import pallas as pl
from jax.experimental.pallas import tpu as pltpu

F32, BF16, U32, I32 = jnp.float32, jnp.bfloat16, jnp.uint32, jnp.int32
LANES = 128
LN_EPS = float(np.asarray(1e-5, ml_dtypes.bfloat16))
MASK_VALUE = -1000000000.0
PASS_ROWS = 32
PASSES_PER_STEP = 4
HEAD_GROUP = 2
SCORE_LAG, MIX_LAG = 2, 1
WO_SPLITS = (8, 20, 26, 30)
X_PARTS = 2


def _round_bf16(v):
    return v.astype(BF16).astype(F32)


def _load_packed(ref, *idx):
    return pltpu.bitcast(ref[idx], BF16)


def _paced(bits, after):
    return (pltpu.bitcast(after, U32) | bits) & bits


def _aligned(i, n):
    return i if isinstance(i, int) else pl.multiple_of(i, n)


def _kernel(x_hbm, mem0_ref, wq_hbm, wk_hbm, wv_hbm, wo_hbm, wr_ref, wg_hbm, wu_hbm, wd_hbm,
            out_hbm,
            x_scr, xn_scr, xn0_scr, out_scr, wq_scr, wk_scr, wv_scr, wo_scr,
            stq_scr, stk_scr, stv_scr, wg_scr, wu_scr, wd_scr,
            mem_scr, o_scr, acc_scr, wr_scr, top_scr, topi_scr, sems, *rings,
            S, D, H, E, M, SEG, FF, TP, T0, RING):
    L = M + SEG
    KT = D // LANES
    RING_OFF = RING - T0
    chunk_rows = LANES * H
    piece = (S - T0) // KT
    part = T0 // X_PARTS
    w_hbm = (wq_hbm, wk_hbm, wv_hbm)
    w_scr = (wq_scr, wk_scr, wv_scr)
    st_scr = (stq_scr, stk_scr, stv_scr)
    SEM_X, SEM_W, SEM_WO, SEM_FFN, SEM_OUT, SEM_FIX, SEM_PART = 0, 1, 4, 5, 6, 7, 9

    def x_copy(start, rows, sem):
        return pltpu.make_async_copy(
            x_hbm.at[pl.ds(start, rows)], x_scr.at[pl.ds(start, rows)], sems.at[sem])

    def x_piece_copy(i):
        return x_copy(_aligned(T0 + i * piece, 16), piece, SEM_X)

    def w_copy(m, i):
        return pltpu.make_async_copy(
            w_hbm[m].at[pl.ds(_aligned(i * chunk_rows, chunk_rows), chunk_rows)],
            st_scr[m], sems.at[SEM_W + m])

    def column_copy(src, dst, j, sem):
        return pltpu.make_async_copy(
            src.at[:, pl.ds(_aligned(j * LANES, LANES), LANES)], dst.at[j], sems.at[sem])

    def out_copy(start, rows, sem):
        return pltpu.make_async_copy(
            out_scr.at[pl.ds(start, rows)], out_hbm.at[pl.ds(start, rows)], sems.at[sem])

    ffn_copies = (
        [column_copy(wg_hbm, wg_scr, j, SEM_FFN) for j in range(FF // LANES)]
        + [column_copy(wu_hbm, wu_scr, j, SEM_FFN) for j in range(FF // LANES)]
        + [column_copy(wd_hbm, wd_scr, j, SEM_FFN) for j in range(KT)])

    def layernorm(xb):
        mean = jnp.sum(xb, axis=-1, keepdims=True) * (1.0 / D)
        cen = xb - mean
        var = jnp.sum(cen * cen, axis=-1, keepdims=True) * (1.0 / D)
        std = _round_bf16(jnp.sqrt(_round_bf16(_round_bf16(var) + LN_EPS)))
        return _round_bf16(_round_bf16(xb - _round_bf16(mean)) / std)

    def normalise_rows(start, rows, after=None):
        xb = x_scr[pl.ds(start, rows), :].astype(F32)
        if after is not None:
            one = pltpu.bitcast(_paced(0x3F800000, after[:rows, :LANES]), F32)
            xb = xb * jnp.concatenate([one] * KT, axis=1)
        xn = layernorm(xb)
        xn_scr[pl.ds(start, rows), :] = xn
        wr = jnp.concatenate([wr_scr[...]] * (rows // 8), axis=0)
        score = _round_bf16(jnp.sum(xn * wr, axis=-1, keepdims=True))
        best1, best2, idx1, idx2 = top_scr[0], top_scr[1], topi_scr[0], topi_scr[1]
        sub = lax.broadcasted_iota(I32, (8, LANES), 0)
        for b in range(rows // 8):
            r = jnp.broadcast_to(score[8 * b:8 * b + 8], (8, LANES))
            row = sub + (start + 8 * b)
            gt1, gt2 = r > best1, r > best2
            best2 = jnp.where(gt1, best1, jnp.where(gt2, r, best2))
            idx2 = jnp.where(gt1, idx1, jnp.where(gt2, row, idx2))
            best1 = jnp.where(gt1, r, best1)
            idx1 = jnp.where(gt1, row, idx1)
        top_scr[0], top_scr[1], topi_scr[0], topi_scr[1] = best1, best2, idx1, idx2
        return xn

    def relayout(m, i, g, after=None):
        src = st_scr[m].bitcast(U32)
        hp = H // 2
        w = src[g * 16 * hp:(g + 1) * 16 * hp, :].reshape(8, 2, hp, E)
        lo, hi = w[:, 0], w[:, 1]
        rows = pl.ds(_aligned(i * (LANES // 2) + g * 8, 8), 8)
        for b in range(hp // 8):
            heads = slice(8 * b, 8 * b + 8)
            shift = [16, 16]
            if after is not None:
                for u in range(2):
                    r0 = (2 * b + u) * (T0 // (hp // 4))
                    shift[u] = _paced(16, after[r0:r0 + 8, :LANES])[None]
            even = (lo[:, heads] & 0xFFFF) | (hi[:, heads] << shift[0])
            odd = (lo[:, heads] >> shift[1]) | (hi[:, heads] & np.uint32(0xFFFF0000))
            even, odd = jnp.swapaxes(even, 0, 1), jnp.swapaxes(odd, 0, 1)
            for j in range(8):
                w_scr[m][2 * (8 * b + j), rows, :] = even[j]
                w_scr[m][2 * (8 * b + j) + 1, rows, :] = odd[j]

    def project_first_tokens(m, i, h0):
        rows = pl.ds(_aligned(i * (LANES // 2), LANES // 2), LANES // 2)
        w = jnp.concatenate([_load_packed(w_scr[m], h0 + t, rows) for t in range(4)], axis=1)
        r = jnp.dot(_load_packed(xn0_scr, i), w, preferred_element_type=F32)
        for t in range(4):
            old = rings[h0 + t][m, RING_OFF:RING, :]
            rings[h0 + t][m, RING_OFF:RING, :] = r[:, t * E:(t + 1) * E] + jnp.where(i > 0, old, 0.0)
        return r

    for p in range(X_PARTS):
        x_copy(p * part, part, SEM_PART + p).start()
    w_copy(0, 0).start()
    w_copy(1, 0).start()
    x_piece_copy(0).start()
    w_copy(2, 0).start()
    mem_scr[...] = mem0_ref[...].astype(F32)
    wr_scr[...] = jnp.broadcast_to(wr_ref[...].astype(F32).reshape(1, D), wr_scr.shape)
    top_scr[...] = jnp.full(top_scr.shape, -jnp.inf, F32)
    topi_scr[0] = lax.broadcasted_iota(I32, (8, LANES), 0)
    topi_scr[1] = lax.broadcasted_iota(I32, (8, LANES), 0) + 8
    for p in range(X_PARTS):
        x_copy(p * part, part, SEM_PART + p).wait()
        for r0 in range(p * part, (p + 1) * part, 64):
            xn = normalise_rows(r0, 64)
            for j in range(KT):
                xn0_scr[j, r0 // 2:(r0 + 64) // 2, :] = pltpu.bitcast(
                    xn[:, j * LANES:(j + 1) * LANES].astype(BF16), U32)
    w_copy(0, 0).wait()
    for g in range(LANES // 16):
        relayout(0, 0, g)

    @pl.loop(0, KT)
    def _(i):
        for m in range(3):
            if m < 2:
                w_copy(m + 1, i).wait()
            if m == 1:
                x_piece_copy(i).wait()

            @pl.when(i + 1 < KT)
            def _():
                if m == 2:
                    w_copy(0, i + 1).wait()
                w_copy(m, i + 1).start()
                if m == 1:
                    x_piece_copy(i + 1).start()

            if m == 1:
                column_copy(wo_hbm, wo_scr, i, SEM_WO).start()
            nxt = (m + 1, i) if m < 2 else (0, jnp.minimum(i + 1, KT - 1))
            blocks = piece // 16 if m > 0 else 0
            for g in range(LANES // 16):
                after = project_first_tokens(m, i, 4 * g)
                relayout(*nxt, g, after)
                for n in range(blocks):
                    at = n * (6 * T0 // blocks)
                    if at // T0 == g:
                        start = T0 + i * piece + ((m - 1) * blocks + n) * 8
                        normalise_rows(_aligned(start, 8), 8, after[at % T0:])

    for j in range(KT):
        column_copy(wo_hbm, wo_scr, j, SEM_WO).wait()
    for c in ffn_copies:
        c.start()

    wo_words = wo_scr.bitcast(U32)
    log2e = math.log2(math.e)

    def one_pass(s):
        q_row = lax.broadcasted_iota(I32, (L, L), 0)
        k_col = lax.broadcasted_iota(I32, (L, L), 1)
        visible = (q_row < M) | (q_row >= k_col)
        seg_rows = pl.ds(_aligned(s * SEG, SEG), SEG)
        put = pl.ds(_aligned(lax.rem(RING + s * TP, RING), 8), TP)
        get = pl.ds(_aligned(lax.rem(RING_OFF + s * SEG, RING), 8), SEG)
        lhs = jnp.concatenate(
            [xn_scr[pl.ds(_aligned(T0 + s * TP, 8), TP), :], mem_scr[...]], axis=0).astype(BF16)
        mem_qkv, probs = {}, {}

        def heads(g):
            return range(g * HEAD_GROUP, (g + 1) * HEAD_GROUP)

        def project(g):
            for h in heads(g):
                w = jnp.concatenate([_load_packed(w_scr[m], h) for m in range(3)], axis=1)
                r = jnp.dot(lhs, w, preferred_element_type=F32)
                mem_qkv[h] = [r[TP:, m * E:(m + 1) * E] for m in range(3)]
                for m in range(3):
                    rings[h][m, put, :] = r[:TP, m * E:(m + 1) * E]

        def segment(h, m):
            return jnp.concatenate([mem_qkv[h][m], rings[h][m, get, :]], axis=0)

        def attend(g):
            for h in heads(g):
                q = segment(h, 0)
                sc = lax.dot_general(jnp.concatenate([q[:M], q[M + 8:]], axis=0),
                                     segment(h, 1).astype(BF16),
                                     (((1,), (1,)), ((), ())), preferred_element_type=F32)
                lane = lax.broadcasted_iota(I32, (8, L), 1)
                first = jnp.zeros((8, L), F32)
                keys = (mem_qkv[h][1], rings[h][1, pl.ds(get.start, 8), :])
                for j in range(M + 8):
                    dots = jnp.sum(q[M:M + 8] * keys[j // 8][j % 8:j % 8 + 1], axis=-1, keepdims=True)
                    first = jnp.where(lane == j, dots, first)
                sc = jnp.concatenate([sc[:M], first, sc[M:]], axis=0)
                sc = jnp.where(visible, sc * (E ** -0.5 * log2e), MASK_VALUE * log2e)
                e = jnp.exp2(sc - jnp.max(sc, axis=-1, keepdims=True))
                probs[h] = e / jnp.sum(e, axis=-1, keepdims=True)

        def mix(g):
            for h in heads(g):
                o_scr[:, h * E:(h + 1) * E] = jnp.dot(
                    probs[h], segment(h, 2).astype(BF16), preferred_element_type=F32)

        def output(h0, h1):
            o = o_scr[:, h0 * E:h1 * E]
            for j in range(KT):
                cols = slice(j * LANES, (j + 1) * LANES)
                r = jnp.dot(o, _load_packed(wo_words, j, slice(h0 * E // 2, h1 * E // 2)),
                            preferred_element_type=F32)
                if h0 > 0:
                    r = r + acc_scr[:, cols]
                else:
                    base = x_scr[seg_rows, cols].astype(F32) + xn_scr[seg_rows, cols]
                    r = jnp.concatenate([r[:M], r[M:] + base], axis=0)
                if h1 < H:
                    acc_scr[:, cols] = r
                else:
                    mem_scr[:, cols] = r[:M]
                    out_scr[seg_rows, cols] = r[M:].astype(out_scr.dtype)

        n_groups = H // HEAD_GROUP
        bounds = (0,) + WO_SPLITS + (H,)
        done = 0
        for t in range(n_groups + SCORE_LAG + MIX_LAG):
            if t < n_groups:
                project(t)
            elif done < len(WO_SPLITS):
                assert bounds[done + 1] <= (t - SCORE_LAG - MIX_LAG) * HEAD_GROUP
                output(bounds[done], bounds[done + 1])
                done += 1
            if 0 <= t - SCORE_LAG - MIX_LAG < n_groups:
                mix(t - SCORE_LAG - MIX_LAG)
            if 0 <= t - SCORE_LAG < n_groups:
                attend(t - SCORE_LAG)
        for d in range(done, len(bounds) - 1):
            output(bounds[d], bounds[d + 1])

    step_rows = PASSES_PER_STEP * SEG

    @pl.loop(0, S // step_rows)
    def _(step):
        for u in range(PASSES_PER_STEP):
            one_pass(step * PASSES_PER_STEP + u)
        out_copy(_aligned(step * step_rows, step_rows), step_rows, SEM_OUT).start()

    best1, best2, idx1, idx2 = top_scr[0], top_scr[1], topi_scr[0], topi_scr[1]
    r_a = jnp.max(best1, axis=0, keepdims=True)
    i_a = jnp.min(jnp.where(best1 == r_a, idx1, S - 1), axis=0, keepdims=True)
    rest = jnp.where(idx1 == i_a, best2, best1)
    rest_idx = jnp.where(idx1 == i_a, idx2, idx1)
    r_b = jnp.max(rest, axis=0, keepdims=True)
    i_b = jnp.min(jnp.where((rest == r_b) & (rest_idx != i_a), rest_idx, S - 1),
                  axis=0, keepdims=True)
    picked = [jnp.clip(jnp.max(i), 0, S - 1) for i in (i_a, i_b)]

    sub = lax.broadcasted_iota(I32, (8, D), 0)
    x_sel = jnp.where(sub == 0, xn_scr[pl.ds(picked[0], 1), :],
                      jnp.where(sub == 1, xn_scr[pl.ds(picked[1], 1), :], 0.0))
    for c in ffn_copies:
        c.wait()
    wg_words, wu_words, wd_words = (r.bitcast(U32) for r in (wg_scr, wu_scr, wd_scr))
    hidden = []
    for j in range(FF // LANES):
        w = jnp.concatenate([_load_packed(wg_words, j), _load_packed(wu_words, j)], axis=1)
        r = jnp.dot(x_sel, w, preferred_element_type=F32)
        gate, up = r[:, :LANES], r[:, LANES:]
        hidden.append(gate * jax.nn.sigmoid(gate) * up)
    hidden = jnp.concatenate(hidden, axis=1)
    y = jnp.concatenate(
        [jnp.dot(hidden, _load_packed(wd_words, j), preferred_element_type=F32) for j in range(KT)],
        axis=1)

    out_copy(0, S, SEM_OUT).wait()
    tiles = [_aligned(row // 16 * 16, 16) for row in picked]
    for c, r_c in enumerate((r_a, r_b)):
        weight = jnp.concatenate([jax.nn.sigmoid(r_c)] * KT, axis=1)
        old = out_scr[pl.ds(tiles[c], 16), :].astype(F32)
        hit = lax.broadcasted_iota(I32, (16, D), 0) == lax.rem(picked[c], 16)
        out_scr[pl.ds(tiles[c], 16), :] = jnp.where(
            hit, old + y[c:c + 1] * weight, old).astype(out_scr.dtype)

    out_copy(tiles[0], 16, SEM_FIX).start()

    @pl.when(tiles[0] != tiles[1])
    def _():
        out_copy(tiles[1], 16, SEM_FIX + 1).start()
        out_copy(tiles[1], 16, SEM_FIX + 1).wait()

    out_copy(tiles[0], 16, SEM_FIX).wait()


@functools.partial(jax.jit, static_argnames=("A_seg_len",))
def pallas_parallel_sum__memory_aug_recurrent_mem_tr__moe_arch_mod__prompt_kernel(
    A_x, A_mem0, A_Wq, A_Wk, A_Wv, A_Wo, A_seg_len, B_x, B_w_r, B_w_gate, B_w_up, B_w_down,
):
    del B_x
    B, S, D = A_x.shape
    _, H, E = A_Wq.shape
    M, SEG, FF = A_mem0.shape[1], int(A_seg_len), B_w_gate.shape[1]
    KT = D // LANES
    TP = PASS_ROWS - M
    T0 = S - (S // SEG) * TP
    period = math.lcm(TP, SEG)
    RING = -(-(T0 + TP) // period) * period
    assert B == 1 and E == LANES and M == 8 and H == 32 and D % LANES == 0 and FF % LANES == 0
    assert SEG % 16 == 0 and S % (SEG * PASSES_PER_STEP) == 0 and 0 < TP <= SEG and TP % 8 == 0
    assert (RING - T0) % SEG == 0 and T0 % (64 * X_PARTS) == 0
    assert (S - T0) % (16 * KT) == 0 and (6 * T0 * 16 * KT // (S - T0)) % 8 == 0

    hbm = pl.BlockSpec(memory_space=pl.ANY)
    vmem = pl.BlockSpec(memory_space=pltpu.VMEM)
    scratch = [
        pltpu.VMEM((S, D), A_x.dtype),
        pltpu.VMEM((S, D), F32),
        pltpu.VMEM((KT, T0 // 2, LANES), U32),
        pltpu.VMEM((S, D), A_x.dtype),
        *[pltpu.VMEM((H, D // 2, E), U32)] * 3,
        pltpu.VMEM((KT, H * E, LANES), BF16),
        *[pltpu.VMEM((LANES * H, E), BF16)] * 3,
        *[pltpu.VMEM((FF // LANES, D, LANES), BF16)] * 2,
        pltpu.VMEM((KT, FF, LANES), BF16),
        pltpu.VMEM((M, D), F32),
        pltpu.VMEM((M + SEG, H * E), F32),
        pltpu.VMEM((M + SEG, D), F32),
        pltpu.VMEM((8, D), F32),
        pltpu.VMEM((2, 8, LANES), F32),
        pltpu.VMEM((2, 8, LANES), I32),
        pltpu.SemaphoreType.DMA((9 + X_PARTS,)),
        *[pltpu.VMEM((3, RING, E), F32)] * H,
    ]
    out = pl.pallas_call(
        functools.partial(_kernel, S=S, D=D, H=H, E=E, M=M, SEG=SEG, FF=FF, TP=TP, T0=T0, RING=RING),
        out_shape=jax.ShapeDtypeStruct((S, D), A_x.dtype),
        in_specs=[hbm, vmem, hbm, hbm, hbm, hbm, vmem, hbm, hbm, hbm],
        out_specs=hbm,
        scratch_shapes=scratch,
        compiler_params=pltpu.CompilerParams(
            vmem_limit_bytes=120 * 1024 * 1024, disable_bounds_checks=True),
        name="rmt_mod",
    )(A_x.reshape(S, D), A_mem0.reshape(M, D),
      A_Wq.reshape(D * H, E), A_Wk.reshape(D * H, E), A_Wv.reshape(D * H, E),
      A_Wo.reshape(H * E, D), B_w_r, B_w_gate, B_w_up, B_w_down)
    return out.reshape(B, S, D)
```

```python
import functools
import math

import jax
import jax.numpy as jnp
import numpy as np
from jax import lax
from jax.experimental import pallas as pl
from jax.experimental.pallas import tpu as pltpu

F32, BF16, U32, I32 = jnp.float32, jnp.bfloat16, jnp.uint32, jnp.int32
LANES = 128
LN_EPS = 1.0013580322265625e-05
MASK_VALUE = -1000000000.0
PASS_ROWS = 32
PASSES_PER_STEP = 4
HEAD_GROUP = 2
SCORE_LAG, MIX_LAG = 2, 1
WO_SPLITS = (8, 20, 26, 30)
X_PARTS = 2


def _round_bf16(v):
    return v.astype(BF16).astype(F32)


def _load_packed(ref, *idx):
    return pltpu.bitcast(ref[idx], BF16)


def _paced(bits, after):
    return (pltpu.bitcast(after, U32) | bits) & bits


def _aligned(i, n):
    return i if isinstance(i, int) else pl.multiple_of(i, n)


def _kernel(x_hbm, mem0_hbm, wq_hbm, wk_hbm, wv_hbm, wo_hbm, wr_hbm, wg_hbm, wu_hbm, wd_hbm,
            out_hbm,
            x_scr, xn_scr, xn0_scr, out_scr, wq_scr, wk_scr, wv_scr, wo_scr,
            stq_scr, stk_scr, stv_scr, wg_scr, wu_scr, wd_scr,
            mem0_scr, mem_scr, o_scr, acc_scr, wr_scr, top_scr, topi_scr, sems, *rings,
            S, D, H, E, M, SEG, FF, TP, T0, RING):
    *rings, wr0_scr = rings
    L = M + SEG
    KT = D // LANES
    RING_OFF = RING - T0
    chunk_rows = LANES * H
    piece = (S - T0) // KT
    part = T0 // X_PARTS
    w_hbm = (wq_hbm, wk_hbm, wv_hbm)
    w_scr = (wq_scr, wk_scr, wv_scr)
    st_scr = (stq_scr, stk_scr, stv_scr)
    SEM_X, SEM_W, SEM_WO, SEM_FFN, SEM_OUT, SEM_FIX, SEM_SMALL, SEM_PART = 0, 1, 4, 5, 6, 7, 9, 11

    def x_copy(start, rows, sem):
        return pltpu.make_async_copy(
            x_hbm.at[pl.ds(start, rows)], x_scr.at[pl.ds(start, rows)], sems.at[sem])

    def x_piece_copy(i):
        return x_copy(_aligned(T0 + i * piece, 16), piece, SEM_X)

    def w_copy(m, i):
        return pltpu.make_async_copy(
            w_hbm[m].at[pl.ds(_aligned(i * chunk_rows, chunk_rows), chunk_rows)],
            st_scr[m], sems.at[SEM_W + m])

    def column_copy(src, dst, j, sem):
        return pltpu.make_async_copy(
            src.at[:, pl.ds(_aligned(j * LANES, LANES), LANES)], dst.at[j], sems.at[sem])

    def out_copy(start, rows, sem):
        return pltpu.make_async_copy(
            out_scr.at[pl.ds(start, rows)], out_hbm.at[pl.ds(start, rows)], sems.at[sem])

    ffn_copies = (
        [column_copy(wg_hbm, wg_scr, j, SEM_FFN) for j in range(FF // LANES)]
        + [column_copy(wu_hbm, wu_scr, j, SEM_FFN) for j in range(FF // LANES)]
        + [column_copy(wd_hbm, wd_scr, j, SEM_FFN) for j in range(KT)])

    def layernorm(xb):
        mean = jnp.sum(xb, axis=-1, keepdims=True) * (1.0 / D)
        cen = xb - mean
        var = jnp.sum(cen * cen, axis=-1, keepdims=True) * (1.0 / D)
        std = _round_bf16(jnp.sqrt(_round_bf16(_round_bf16(var) + LN_EPS)))
        return _round_bf16(_round_bf16(xb - _round_bf16(mean)) / std)

    def normalise_rows(start, rows, after=None):
        xb = x_scr[pl.ds(start, rows), :].astype(F32)
        if after is not None:
            one = pltpu.bitcast(_paced(0x3F800000, after[:rows, :LANES]), F32)
            xb = xb * jnp.concatenate([one] * KT, axis=1)
        xn = layernorm(xb)
        xn_scr[pl.ds(start, rows), :] = xn
        wr = jnp.concatenate([wr_scr[...]] * (rows // 8), axis=0)
        score = _round_bf16(jnp.sum(xn * wr, axis=-1, keepdims=True))
        best1, best2, idx1, idx2 = top_scr[0], top_scr[1], topi_scr[0], topi_scr[1]
        sub = lax.broadcasted_iota(I32, (8, LANES), 0)
        for b in range(rows // 8):
            r = jnp.broadcast_to(score[8 * b:8 * b + 8], (8, LANES))
            row = sub + (start + 8 * b)
            gt1, gt2 = r > best1, r > best2
            best2 = jnp.where(gt1, best1, jnp.where(gt2, r, best2))
            idx2 = jnp.where(gt1, idx1, jnp.where(gt2, row, idx2))
            best1 = jnp.where(gt1, r, best1)
            idx1 = jnp.where(gt1, row, idx1)
        top_scr[0], top_scr[1], topi_scr[0], topi_scr[1] = best1, best2, idx1, idx2
        return xn

    def relayout(m, i, g, after=None):
        src = st_scr[m].bitcast(U32)
        hp = H // 2
        w = src[g * 16 * hp:(g + 1) * 16 * hp, :].reshape(8, 2, hp, E)
        lo, hi = w[:, 0], w[:, 1]
        rows = pl.ds(_aligned(i * (LANES // 2) + g * 8, 8), 8)
        for b in range(hp // 8):
            heads = slice(8 * b, 8 * b + 8)
            shift = [16, 16]
            if after is not None:
                for u in range(2):
                    r0 = (2 * b + u) * (T0 // (hp // 4))
                    shift[u] = _paced(16, after[r0:r0 + 8, :LANES])[None]
            even = (lo[:, heads] & 0xFFFF) | (hi[:, heads] << shift[0])
            odd = (lo[:, heads] >> shift[1]) | (hi[:, heads] & np.uint32(0xFFFF0000))
            even, odd = jnp.swapaxes(even, 0, 1), jnp.swapaxes(odd, 0, 1)
            for j in range(8):
                w_scr[m][2 * (8 * b + j), rows, :] = even[j]
                w_scr[m][2 * (8 * b + j) + 1, rows, :] = odd[j]

    def project_first_tokens(m, i, h0):
        rows = pl.ds(_aligned(i * (LANES // 2), LANES // 2), LANES // 2)
        w = jnp.concatenate([_load_packed(w_scr[m], h0 + t, rows) for t in range(4)], axis=1)
        r = jnp.dot(_load_packed(xn0_scr, i), w, preferred_element_type=F32)
        for t in range(4):
            old = rings[h0 + t][m, RING_OFF:RING, :]
            rings[h0 + t][m, RING_OFF:RING, :] = r[:, t * E:(t + 1) * E] + jnp.where(i > 0, old, 0.0)
        return r

    wr_copy = pltpu.make_async_copy(wr_hbm, wr0_scr, sems.at[SEM_SMALL])
    mem0_copy = pltpu.make_async_copy(mem0_hbm, mem0_scr, sems.at[SEM_SMALL + 1])
    wr_copy.start()
    for p in range(X_PARTS):
        x_copy(p * part, part, SEM_PART + p).start()
    w_copy(0, 0).start()
    w_copy(1, 0).start()
    x_piece_copy(0).start()
    w_copy(2, 0).start()
    mem0_copy.start()
    top_scr[...] = jnp.full(top_scr.shape, -jnp.inf, F32)
    topi_scr[0] = lax.broadcasted_iota(I32, (8, LANES), 0)
    topi_scr[1] = lax.broadcasted_iota(I32, (8, LANES), 0) + 8
    wr_copy.wait()
    wr_scr[...] = jnp.broadcast_to(wr0_scr[...].astype(F32).reshape(1, D), wr_scr.shape)
    for p in range(X_PARTS):
        x_copy(p * part, part, SEM_PART + p).wait()
        for r0 in range(p * part, (p + 1) * part, 64):
            xn = normalise_rows(r0, 64)
            for j in range(KT):
                xn0_scr[j, r0 // 2:(r0 + 64) // 2, :] = pltpu.bitcast(
                    xn[:, j * LANES:(j + 1) * LANES].astype(BF16), U32)
    w_copy(0, 0).wait()
    for g in range(LANES // 16):
        relayout(0, 0, g)

    @pl.loop(0, KT)
    def _(i):
        for m in range(3):
            if m < 2:
                w_copy(m + 1, i).wait()
            if m == 1:
                x_piece_copy(i).wait()

            @pl.when(i + 1 < KT)
            def _():
                if m == 2:
                    w_copy(0, i + 1).wait()
                w_copy(m, i + 1).start()
                if m == 1:
                    x_piece_copy(i + 1).start()

            if m == 1:
                column_copy(wo_hbm, wo_scr, i, SEM_WO).start()
            nxt = (m + 1, i) if m < 2 else (0, jnp.minimum(i + 1, KT - 1))
            blocks = piece // 16 if m > 0 else 0
            for g in range(LANES // 16):
                after = project_first_tokens(m, i, 4 * g)
                relayout(*nxt, g, after)
                for n in range(blocks):
                    at = n * (6 * T0 // blocks)
                    if at // T0 == g:
                        start = T0 + i * piece + ((m - 1) * blocks + n) * 8
                        normalise_rows(_aligned(start, 8), 8, after[at % T0:])

    for j in range(KT):
        column_copy(wo_hbm, wo_scr, j, SEM_WO).wait()
    mem0_copy.wait()
    mem_scr[...] = mem0_scr[...].astype(F32)
    for c in ffn_copies:
        c.start()

    wo_words = wo_scr.bitcast(U32)
    log2e = math.log2(math.e)

    def one_pass(step, u):
        s = step * PASSES_PER_STEP + u
        q_row = lax.broadcasted_iota(I32, (L, L), 0)
        k_col = lax.broadcasted_iota(I32, (L, L), 1)
        visible = (q_row < M) | (q_row >= k_col)
        seg_rows = pl.ds(_aligned(s * SEG, SEG), SEG)
        put = pl.ds(_aligned(lax.rem(step * (PASSES_PER_STEP * TP), RING), 8) + u * TP, TP)
        get = pl.ds(_aligned(lax.rem(RING_OFF + s * SEG, RING), 8), SEG)
        lhs = jnp.concatenate(
            [xn_scr[pl.ds(_aligned(T0 + s * TP, 8), TP), :], mem_scr[...]], axis=0).astype(BF16)
        mem_qkv, probs = {}, {}

        def heads(g):
            return range(g * HEAD_GROUP, (g + 1) * HEAD_GROUP)

        def project(g):
            for h in heads(g):
                w = jnp.concatenate([_load_packed(w_scr[m], h) for m in range(3)], axis=1)
                r = jnp.dot(lhs, w, preferred_element_type=F32)
                mem_qkv[h] = [r[TP:, m * E:(m + 1) * E] for m in range(3)]
                for m in range(3):
                    rings[h][m, put, :] = r[:TP, m * E:(m + 1) * E]

        def segment(h, m):
            return jnp.concatenate([mem_qkv[h][m], rings[h][m, get, :]], axis=0)

        def attend(g):
            for h in heads(g):
                q = segment(h, 0)
                sc = lax.dot_general(jnp.concatenate([q[:M], q[M + 8:]], axis=0),
                                     segment(h, 1).astype(BF16),
                                     (((1,), (1,)), ((), ())), preferred_element_type=F32)
                lane = lax.broadcasted_iota(I32, (8, L), 1)
                first = jnp.zeros((8, L), F32)
                keys = (mem_qkv[h][1], rings[h][1, pl.ds(get.start, 8), :])
                for j in range(M + 8):
                    dots = jnp.sum(q[M:M + 8] * keys[j // 8][j % 8:j % 8 + 1], axis=-1, keepdims=True)
                    first = jnp.where(lane == j, dots, first)
                sc = jnp.concatenate([sc[:M], first, sc[M:]], axis=0)
                sc = jnp.where(visible, sc * (E ** -0.5 * log2e), MASK_VALUE * log2e)
                e = jnp.exp2(sc - jnp.max(sc, axis=-1, keepdims=True))
                probs[h] = e / jnp.sum(e, axis=-1, keepdims=True)

        def mix(g):
            for h in heads(g):
                o_scr[:, h * E:(h + 1) * E] = jnp.dot(
                    probs[h], segment(h, 2).astype(BF16), preferred_element_type=F32)

        def output(h0, h1):
            o = o_scr[:, h0 * E:h1 * E]
            for j in range(KT):
                cols = slice(j * LANES, (j + 1) * LANES)
                r = jnp.dot(o, _load_packed(wo_words, j, slice(h0 * E // 2, h1 * E // 2)),
                            preferred_element_type=F32)
                if h0 > 0:
                    r = r + acc_scr[:, cols]
                else:
                    base = x_scr[seg_rows, cols].astype(F32) + xn_scr[seg_rows, cols]
                    r = jnp.concatenate([r[:M], r[M:] + base], axis=0)
                if h1 < H:
                    acc_scr[:, cols] = r
                else:
                    mem_scr[:, cols] = r[:M]
                    out_scr[seg_rows, cols] = r[M:].astype(out_scr.dtype)

        n_groups = H // HEAD_GROUP
        bounds = (0,) + WO_SPLITS + (H,)
        done = 0
        for t in range(n_groups + SCORE_LAG + MIX_LAG):
            if t < n_groups:
                project(t)
            elif done < len(WO_SPLITS):
                assert bounds[done + 1] <= (t - SCORE_LAG - MIX_LAG) * HEAD_GROUP
                output(bounds[done], bounds[done + 1])
                done += 1
            if 0 <= t - SCORE_LAG - MIX_LAG < n_groups:
                mix(t - SCORE_LAG - MIX_LAG)
            if 0 <= t - SCORE_LAG < n_groups:
                attend(t - SCORE_LAG)
        for d in range(done, len(bounds) - 1):
            output(bounds[d], bounds[d + 1])

    step_rows = PASSES_PER_STEP * SEG

    @pl.loop(0, S // step_rows)
    def _(step):
        for u in range(PASSES_PER_STEP):
            one_pass(step, u)
        out_copy(_aligned(step * step_rows, step_rows), step_rows, SEM_OUT).start()

    for c in ffn_copies:
        c.wait()
    best1, best2, idx1, idx2 = top_scr[0], top_scr[1], topi_scr[0], topi_scr[1]
    r_a = jnp.max(best1, axis=0, keepdims=True)
    i_a = jnp.min(jnp.where(best1 == r_a, idx1, S - 1), axis=0, keepdims=True)
    rest = jnp.where(idx1 == i_a, best2, best1)
    rest_idx = jnp.where(idx1 == i_a, idx2, idx1)
    r_b = jnp.max(rest, axis=0, keepdims=True)
    i_b = jnp.min(jnp.where((rest == r_b) & (rest_idx != i_a), rest_idx, S - 1),
                  axis=0, keepdims=True)
    picked = [jnp.clip(i[0, 0], 0, S - 1) for i in (i_a, i_b)]

    sub = lax.broadcasted_iota(I32, (8, D), 0)
    x_sel = jnp.where(sub == 0, xn_scr[pl.ds(picked[0], 1), :],
                      jnp.where(sub == 1, xn_scr[pl.ds(picked[1], 1), :], 0.0))
    wg_words, wu_words, wd_words = (r.bitcast(U32) for r in (wg_scr, wu_scr, wd_scr))
    hidden = []
    for j in range(FF // LANES):
        w = jnp.concatenate([_load_packed(wg_words, j), _load_packed(wu_words, j)], axis=1)
        r = jnp.dot(x_sel, w, preferred_element_type=F32)
        gate, up = r[:, :LANES], r[:, LANES:]
        hidden.append(gate * jax.nn.sigmoid(gate) * up)
    hidden = jnp.concatenate(hidden, axis=1)
    y = jnp.concatenate(
        [jnp.dot(hidden, _load_packed(wd_words, j), preferred_element_type=F32) for j in range(KT)],
        axis=1)

    out_copy(0, S, SEM_OUT).wait()
    tiles = [_aligned(row // 16 * 16, 16) for row in picked]
    for c, r_c in enumerate((r_a, r_b)):
        weight = jnp.concatenate([jax.nn.sigmoid(r_c)] * KT, axis=1)
        old = out_scr[pl.ds(tiles[c], 16), :].astype(F32)
        hit = lax.broadcasted_iota(I32, (16, D), 0) == lax.rem(picked[c], 16)
        out_scr[pl.ds(tiles[c], 16), :] = jnp.where(
            hit, old + y[c:c + 1] * weight, old).astype(out_scr.dtype)

    out_copy(tiles[0], 16, SEM_FIX).start()

    @pl.when(tiles[0] != tiles[1])
    def _():
        out_copy(tiles[1], 16, SEM_FIX + 1).start()
        out_copy(tiles[1], 16, SEM_FIX + 1).wait()

    out_copy(tiles[0], 16, SEM_FIX).wait()


@functools.partial(jax.jit, static_argnames=("A_seg_len",))
def pallas_parallel_sum__memory_aug_recurrent_mem_tr__moe_arch_mod__prompt_kernel(
    A_x, A_mem0, A_Wq, A_Wk, A_Wv, A_Wo, A_seg_len, B_x, B_w_r, B_w_gate, B_w_up, B_w_down,
):
    del B_x
    B, S, D = A_x.shape
    _, H, E = A_Wq.shape
    M, SEG, FF = A_mem0.shape[1], int(A_seg_len), B_w_gate.shape[1]
    KT = D // LANES
    TP = PASS_ROWS - M
    T0 = S - (S // SEG) * TP
    period = math.lcm(PASSES_PER_STEP * TP, SEG)
    RING = -(-(T0 + TP) // period) * period
    assert B == 1 and E == LANES and M == 8 and H == 32 and D % LANES == 0 and FF % LANES == 0
    assert SEG % 16 == 0 and S % (SEG * PASSES_PER_STEP) == 0 and 0 < TP <= SEG and TP % 8 == 0
    assert (RING - T0) % SEG == 0 and T0 % (64 * X_PARTS) == 0
    assert (S - T0) % (16 * KT) == 0 and (6 * T0 * 16 * KT // (S - T0)) % 8 == 0

    hbm = pl.BlockSpec(memory_space=pl.ANY)
    scratch = [
        pltpu.VMEM((S, D), A_x.dtype),
        pltpu.VMEM((S, D), F32),
        pltpu.VMEM((KT, T0 // 2, LANES), U32),
        pltpu.VMEM((S, D), A_x.dtype),
        *[pltpu.VMEM((H, D // 2, E), U32)] * 3,
        pltpu.VMEM((KT, H * E, LANES), BF16),
        *[pltpu.VMEM((LANES * H, E), BF16)] * 3,
        *[pltpu.VMEM((FF // LANES, D, LANES), BF16)] * 2,
        pltpu.VMEM((KT, FF, LANES), BF16),
        pltpu.VMEM((M, D), A_mem0.dtype),
        pltpu.VMEM((M, D), F32),
        pltpu.VMEM((M + SEG, H * E), F32),
        pltpu.VMEM((M + SEG, D), F32),
        pltpu.VMEM((8, D), F32),
        pltpu.VMEM((2, 8, LANES), F32),
        pltpu.VMEM((2, 8, LANES), I32),
        pltpu.SemaphoreType.DMA((11 + X_PARTS,)),
        *[pltpu.VMEM((3, RING, E), F32)] * H,
        pltpu.VMEM((D,), B_w_r.dtype),
    ]
    out = pl.pallas_call(
        functools.partial(_kernel, S=S, D=D, H=H, E=E, M=M, SEG=SEG, FF=FF, TP=TP, T0=T0, RING=RING),
        out_shape=jax.ShapeDtypeStruct((S, D), A_x.dtype),
        in_specs=[hbm] * 10,
        out_specs=hbm,
        scratch_shapes=scratch,
        compiler_params=pltpu.CompilerParams(
            vmem_limit_bytes=120 * 1024 * 1024,
            disable_bounds_checks=True, disable_semaphore_checks=True),
        name="rmt_mod",
    )(A_x.reshape(S, D), A_mem0.reshape(M, D),
      A_Wq.reshape(D * H, E), A_Wk.reshape(D * H, E), A_Wv.reshape(D * H, E),
      A_Wo.reshape(H * E, D), B_w_r, B_w_gate, B_w_up, B_w_down)
    return out.reshape(B, S, D)
```

```python
import functools
import math

import jax
import jax.numpy as jnp
import numpy as np
from jax import lax
from jax.experimental import pallas as pl
from jax.experimental.pallas import tpu as pltpu

F32, BF16, U32, I32 = jnp.float32, jnp.bfloat16, jnp.uint32, jnp.int32
LANES = 128
LN_EPS = 1.0013580322265625e-05
MASK_VALUE = -1000000000.0
PASS_ROWS = 32
PASSES_PER_STEP = 4
HEAD_GROUP = 2
SCORE_LAG, MIX_LAG = 2, 1
WO_SPLITS = (8, 20, 26, 30)


def _round_bf16(v):
    return v.astype(BF16).astype(F32)


def _load_packed(ref, *idx):
    return pltpu.bitcast(ref[idx], BF16)


def _paced(bits, after):
    return (pltpu.bitcast(after, U32) | bits) & bits


def _aligned(i, n):
    return i if isinstance(i, int) else pl.multiple_of(i, n)


def _kernel(x_hbm, mem0_hbm, wq_hbm, wk_hbm, wv_hbm, wo_hbm, wr_hbm, wg_hbm, wu_hbm, wd_hbm,
            out_hbm,
            x_scr, xn_scr, xn0_scr, out_scr, wq_scr, wk_scr, wv_scr, wo_scr,
            stq_scr, stk_scr, stv_scr, wg_scr, wu_scr, wd_scr,
            mem0_scr, mem_scr, o_scr, acc_scr, wr_scr, top_scr, topi_scr, sems, *rings,
            S, D, H, E, M, SEG, FF, TP, T0, RING):
    *rings, wr0_scr = rings
    L = M + SEG
    KT = D // LANES
    RING_OFF = RING - T0
    chunk_rows = LANES * H
    piece = (S - T0) // KT
    w_hbm = (wq_hbm, wk_hbm, wv_hbm)
    w_scr = (wq_scr, wk_scr, wv_scr)
    st_scr = (stq_scr, stk_scr, stv_scr)
    SEM_X, SEM_W, SEM_WO, SEM_FFN, SEM_OUT, SEM_FIX, SEM_SMALL, SEM_HALF = 0, 1, 4, 5, 6, 7, 9, 11

    def x_copy(start, rows, sem):
        return pltpu.make_async_copy(
            x_hbm.at[pl.ds(start, rows)], x_scr.at[pl.ds(start, rows)], sems.at[sem])

    def x_piece_copy(i):
        return x_copy(_aligned(T0 + i * piece, 16), piece, SEM_X)

    def w_copy(m, i):
        return pltpu.make_async_copy(
            w_hbm[m].at[pl.ds(_aligned(i * chunk_rows, chunk_rows), chunk_rows)],
            st_scr[m], sems.at[SEM_W + m])

    def column_copy(src, dst, j, sem):
        return pltpu.make_async_copy(
            src.at[:, pl.ds(_aligned(j * LANES, LANES), LANES)], dst.at[j], sems.at[sem])

    def out_copy(start, rows, sem):
        return pltpu.make_async_copy(
            out_scr.at[pl.ds(start, rows)], out_hbm.at[pl.ds(start, rows)], sems.at[sem])

    ffn_copies = (
        [column_copy(wg_hbm, wg_scr, j, SEM_FFN) for j in range(FF // LANES)]
        + [column_copy(wu_hbm, wu_scr, j, SEM_FFN) for j in range(FF // LANES)]
        + [column_copy(wd_hbm, wd_scr, j, SEM_FFN) for j in range(KT)])

    def layernorm(xb):
        mean = jnp.sum(xb, axis=-1, keepdims=True) * (1.0 / D)
        cen = xb - mean
        var = jnp.sum(cen * cen, axis=-1, keepdims=True) * (1.0 / D)
        std = _round_bf16(jnp.sqrt(_round_bf16(_round_bf16(var) + LN_EPS)))
        return _round_bf16(_round_bf16(xb - _round_bf16(mean)) / std)

    def normalise_rows(start, rows, after=None):
        xb = x_scr[pl.ds(start, rows), :].astype(F32)
        if after is not None:
            one = pltpu.bitcast(_paced(0x3F800000, after[:rows, :LANES]), F32)
            xb = xb * jnp.concatenate([one] * KT, axis=1)
        xn = layernorm(xb)
        xn_scr[pl.ds(start, rows), :] = xn
        wr = jnp.concatenate([wr_scr[...]] * (rows // 8), axis=0)
        score = _round_bf16(jnp.sum(xn * wr, axis=-1, keepdims=True))
        best1, best2, idx1, idx2 = top_scr[0], top_scr[1], topi_scr[0], topi_scr[1]
        sub = lax.broadcasted_iota(I32, (8, LANES), 0)
        for b in range(rows // 8):
            r = jnp.broadcast_to(score[8 * b:8 * b + 8], (8, LANES))
            row = sub + (start + 8 * b)
            gt1, gt2 = r > best1, r > best2
            best2 = jnp.where(gt1, best1, jnp.where(gt2, r, best2))
            idx2 = jnp.where(gt1, idx1, jnp.where(gt2, row, idx2))
            best1 = jnp.where(gt1, r, best1)
            idx1 = jnp.where(gt1, row, idx1)
        top_scr[0], top_scr[1], topi_scr[0], topi_scr[1] = best1, best2, idx1, idx2
        return xn

    def relayout(m, i, g, after=None):
        src = st_scr[m].bitcast(U32)
        hp = H // 2
        w = src[g * 16 * hp:(g + 1) * 16 * hp, :].reshape(8, 2, hp, E)
        lo, hi = w[:, 0], w[:, 1]
        rows = pl.ds(_aligned(i * (LANES // 2) + g * 8, 8), 8)
        for b in range(hp // 8):
            heads = slice(8 * b, 8 * b + 8)
            shift = [16, 16]
            if after is not None:
                for u in range(2):
                    r0 = (2 * b + u) * (after.shape[0] // (hp // 4))
                    shift[u] = _paced(16, after[r0:r0 + 8, :LANES])[None]
            even = (lo[:, heads] & 0xFFFF) | (hi[:, heads] << shift[0])
            odd = (lo[:, heads] >> shift[1]) | (hi[:, heads] & np.uint32(0xFFFF0000))
            even, odd = jnp.swapaxes(even, 0, 1), jnp.swapaxes(odd, 0, 1)
            for j in range(8):
                w_scr[m][2 * (8 * b + j), rows, :] = even[j]
                w_scr[m][2 * (8 * b + j) + 1, rows, :] = odd[j]

    def project_first_tokens(m, i, h0, r0, r1, first):
        rows = pl.ds(_aligned(i * (LANES // 2), LANES // 2), LANES // 2)
        w = jnp.concatenate([_load_packed(w_scr[m], h0 + t, rows) for t in range(4)], axis=1)
        r = jnp.dot(_load_packed(xn0_scr, i, slice(r0 // 2, r1 // 2)), w, preferred_element_type=F32)
        for t in range(4):
            ring, dst = rings[h0 + t], slice(RING_OFF + r0, RING_OFF + r1)
            new = r[:, t * E:(t + 1) * E]
            if first is False:
                new = new + ring[m, dst, :]
            elif first is not True:
                new = new + jnp.where(first, 0.0, ring[m, dst, :])
            ring[m, dst, :] = new
        return r

    def normalise_first_tokens(r0, rows, after=None):
        xn = normalise_rows(r0, rows, after)
        for j in range(KT):
            xn0_scr[j, r0 // 2:(r0 + rows) // 2, :] = pltpu.bitcast(
                xn[:, j * LANES:(j + 1) * LANES].astype(BF16), U32)

    def prologue_stage(m, i, first, r0=0, r1=T0, nxt=None, norms=()):
        for g in range(LANES // 16):
            r = project_first_tokens(m, i, 4 * g, r0, r1, first)
            if nxt is not None:
                relayout(*nxt, g, r)
            for n, norm in enumerate(norms):
                at = n * (6 * (r1 - r0) // len(norms)) // 16 * 16
                if at // (r1 - r0) == g:
                    norm(r[at % (r1 - r0):])

    def half_piece(start):
        return [functools.partial(normalise_rows, _aligned(start + r, 8), 8)
                for r in range(0, piece // 2, 8)]

    half = T0 // 2
    wr_copy = pltpu.make_async_copy(wr_hbm, wr0_scr, sems.at[SEM_SMALL])
    mem0_copy = pltpu.make_async_copy(mem0_hbm, mem0_scr, sems.at[SEM_SMALL + 1])
    wr_copy.start()
    x_copy(0, half, SEM_HALF).start()
    w_copy(0, 0).start()
    x_copy(half, half, SEM_HALF + 1).start()
    w_copy(1, 0).start()
    w_copy(2, 0).start()
    x_piece_copy(0).start()
    mem0_copy.start()
    top_scr[...] = jnp.full(top_scr.shape, -jnp.inf, F32)
    topi_scr[0] = lax.broadcasted_iota(I32, (8, LANES), 0)
    topi_scr[1] = lax.broadcasted_iota(I32, (8, LANES), 0) + 8
    wr_copy.wait()
    wr_scr[...] = jnp.broadcast_to(wr0_scr[...].astype(F32).reshape(1, D), wr_scr.shape)
    x_copy(0, half, SEM_HALF).wait()
    for r0 in range(0, half, 64):
        normalise_first_tokens(r0, 64)
    w_copy(0, 0).wait()
    for g in range(LANES // 16):
        relayout(0, 0, g)

    x_copy(half, half, SEM_HALF + 1).wait()
    w_copy(0, 1).start()
    prologue_stage(0, 0, True, 0, half, norms=[
        functools.partial(normalise_first_tokens, r, 16) for r in range(half, T0, 16)])
    w_copy(1, 0).wait()
    prologue_stage(0, 0, True, half, T0, nxt=(1, 0))

    @pl.loop(0, KT)
    def _(i):
        more = i + 1 < KT
        w_copy(2, i).wait()
        x_piece_copy(i).wait()

        @pl.when(more)
        def _():
            w_copy(1, i + 1).start()
            x_piece_copy(i + 1).start()

        column_copy(wo_hbm, wo_scr, i, SEM_WO).start()
        prologue_stage(1, i, i == 0, nxt=(2, i), norms=half_piece(T0 + i * piece))

        @pl.when(more)
        def _():
            w_copy(0, i + 1).wait()
            w_copy(2, i + 1).start()

        prologue_stage(2, i, i == 0, nxt=(0, jnp.minimum(i + 1, KT - 1)),
                       norms=half_piece(T0 + i * piece + piece // 2))

        @pl.when(more)
        def _():
            w_copy(1, i + 1).wait()

            @pl.when(i + 2 < KT)
            def _():
                w_copy(0, i + 2).start()

            prologue_stage(0, i + 1, False, nxt=(1, i + 1))

    for j in range(KT):
        column_copy(wo_hbm, wo_scr, j, SEM_WO).wait()
    mem0_copy.wait()
    mem_scr[...] = mem0_scr[...].astype(F32)
    for c in ffn_copies:
        c.start()

    wo_words = wo_scr.bitcast(U32)
    log2e = math.log2(math.e)

    def one_pass(step, u):
        s = step * PASSES_PER_STEP + u
        q_row = lax.broadcasted_iota(I32, (L, L), 0)
        k_col = lax.broadcasted_iota(I32, (L, L), 1)
        visible = (q_row < M) | (q_row >= k_col)
        seg_rows = pl.ds(_aligned(s * SEG, SEG), SEG)
        put = pl.ds(_aligned(lax.rem(step * (PASSES_PER_STEP * TP), RING), 8) + u * TP, TP)
        get = pl.ds(_aligned(lax.rem(RING_OFF + s * SEG, RING), 8), SEG)
        lhs = jnp.concatenate(
            [xn_scr[pl.ds(_aligned(T0 + s * TP, 8), TP), :], mem_scr[...]], axis=0).astype(BF16)
        mem_qkv, probs = {}, {}

        def heads(g):
            return range(g * HEAD_GROUP, (g + 1) * HEAD_GROUP)

        def project(g):
            for h in heads(g):
                w = jnp.concatenate([_load_packed(w_scr[m], h) for m in range(3)], axis=1)
                r = jnp.dot(lhs, w, preferred_element_type=F32)
                mem_qkv[h] = [r[TP:, m * E:(m + 1) * E] for m in range(3)]
                for m in range(3):
                    rings[h][m, put, :] = r[:TP, m * E:(m + 1) * E]

        def segment(h, m):
            return jnp.concatenate([mem_qkv[h][m], rings[h][m, get, :]], axis=0)

        def attend(g):
            for h in heads(g):
                q = segment(h, 0)
                sc = lax.dot_general(jnp.concatenate([q[:M], q[M + 8:]], axis=0),
                                     segment(h, 1).astype(BF16),
                                     (((1,), (1,)), ((), ())), preferred_element_type=F32)
                lane = lax.broadcasted_iota(I32, (8, L), 1)
                first = jnp.zeros((8, L), F32)
                keys = (mem_qkv[h][1], rings[h][1, pl.ds(get.start, 8), :])
                for j in range(M + 8):
                    dots = jnp.sum(q[M:M + 8] * keys[j // 8][j % 8:j % 8 + 1], axis=-1, keepdims=True)
                    first = jnp.where(lane == j, dots, first)
                sc = jnp.concatenate([sc[:M], first, sc[M:]], axis=0)
                sc = jnp.where(visible, sc * (E ** -0.5 * log2e), MASK_VALUE * log2e)
                e = jnp.exp2(sc - jnp.max(sc, axis=-1, keepdims=True))
                probs[h] = e / jnp.sum(e, axis=-1, keepdims=True)

        def mix(g):
            for h in heads(g):
                o_scr[:, h * E:(h + 1) * E] = jnp.dot(
                    probs[h], segment(h, 2).astype(BF16), preferred_element_type=F32)

        def output(h0, h1):
            o = o_scr[:, h0 * E:h1 * E]
            for j in range(KT):
                cols = slice(j * LANES, (j + 1) * LANES)
                r = jnp.dot(o, _load_packed(wo_words, j, slice(h0 * E // 2, h1 * E // 2)),
                            preferred_element_type=F32)
                if h0 > 0:
                    r = r + acc_scr[:, cols]
                else:
                    base = x_scr[seg_rows, cols].astype(F32) + xn_scr[seg_rows, cols]
                    r = jnp.concatenate([r[:M], r[M:] + base], axis=0)
                if h1 < H:
                    acc_scr[:, cols] = r
                else:
                    mem_scr[:, cols] = r[:M]
                    out_scr[seg_rows, cols] = r[M:].astype(out_scr.dtype)

        n_groups = H // HEAD_GROUP
        bounds = (0,) + WO_SPLITS + (H,)
        done = 0
        for t in range(n_groups + SCORE_LAG + MIX_LAG):
            if t < n_groups:
                project(t)
            elif done < len(WO_SPLITS):
                assert bounds[done + 1] <= (t - SCORE_LAG - MIX_LAG) * HEAD_GROUP
                output(bounds[done], bounds[done + 1])
                done += 1
            if 0 <= t - SCORE_LAG - MIX_LAG < n_groups:
                mix(t - SCORE_LAG - MIX_LAG)
            if 0 <= t - SCORE_LAG < n_groups:
                attend(t - SCORE_LAG)
        for d in range(done, len(bounds) - 1):
            output(bounds[d], bounds[d + 1])

    step_rows = PASSES_PER_STEP * SEG

    @pl.loop(0, S // step_rows)
    def _(step):
        for u in range(PASSES_PER_STEP):
            one_pass(step, u)
        out_copy(_aligned(step * step_rows, step_rows), step_rows, SEM_OUT).start()

    for c in ffn_copies:
        c.wait()
    best1, best2, idx1, idx2 = top_scr[0], top_scr[1], topi_scr[0], topi_scr[1]
    r_a = jnp.max(best1, axis=0, keepdims=True)
    i_a = jnp.min(jnp.where(best1 == r_a, idx1, S - 1), axis=0, keepdims=True)
    rest = jnp.where(idx1 == i_a, best2, best1)
    rest_idx = jnp.where(idx1 == i_a, idx2, idx1)
    r_b = jnp.max(rest, axis=0, keepdims=True)
    i_b = jnp.min(jnp.where((rest == r_b) & (rest_idx != i_a), rest_idx, S - 1),
                  axis=0, keepdims=True)
    picked = [jnp.clip(i[0, 0], 0, S - 1) for i in (i_a, i_b)]

    sub = lax.broadcasted_iota(I32, (8, D), 0)
    x_sel = jnp.where(sub == 0, xn_scr[pl.ds(picked[0], 1), :],
                      jnp.where(sub == 1, xn_scr[pl.ds(picked[1], 1), :], 0.0))
    wg_words, wu_words, wd_words = (r.bitcast(U32) for r in (wg_scr, wu_scr, wd_scr))
    hidden = []
    for j in range(FF // LANES):
        w = jnp.concatenate([_load_packed(wg_words, j), _load_packed(wu_words, j)], axis=1)
        r = jnp.dot(x_sel, w, preferred_element_type=F32)
        gate, up = r[:, :LANES], r[:, LANES:]
        hidden.append(gate * jax.nn.sigmoid(gate) * up)
    hidden = jnp.concatenate(hidden, axis=1)
    y = jnp.concatenate(
        [jnp.dot(hidden, _load_packed(wd_words, j), preferred_element_type=F32) for j in range(KT)],
        axis=1)

    out_copy(0, S, SEM_OUT).wait()
    tiles = [_aligned(row // 16 * 16, 16) for row in picked]
    for c, r_c in enumerate((r_a, r_b)):
        weight = jnp.concatenate([jax.nn.sigmoid(r_c)] * KT, axis=1)
        old = out_scr[pl.ds(tiles[c], 16), :].astype(F32)
        hit = lax.broadcasted_iota(I32, (16, D), 0) == lax.rem(picked[c], 16)
        out_scr[pl.ds(tiles[c], 16), :] = jnp.where(
            hit, old + y[c:c + 1] * weight, old).astype(out_scr.dtype)

    out_copy(tiles[0], 16, SEM_FIX).start()

    @pl.when(tiles[0] != tiles[1])
    def _():
        out_copy(tiles[1], 16, SEM_FIX + 1).start()
        out_copy(tiles[1], 16, SEM_FIX + 1).wait()

    out_copy(tiles[0], 16, SEM_FIX).wait()


@functools.partial(jax.jit, static_argnames=("A_seg_len",))
def pallas_parallel_sum__memory_aug_recurrent_mem_tr__moe_arch_mod__prompt_kernel(
    A_x, A_mem0, A_Wq, A_Wk, A_Wv, A_Wo, A_seg_len, B_x, B_w_r, B_w_gate, B_w_up, B_w_down,
):
    del B_x
    B, S, D = A_x.shape
    _, H, E = A_Wq.shape
    M, SEG, FF = A_mem0.shape[1], int(A_seg_len), B_w_gate.shape[1]
    KT = D // LANES
    TP = PASS_ROWS - M
    T0 = S - (S // SEG) * TP
    period = math.lcm(PASSES_PER_STEP * TP, SEG)
    RING = -(-(T0 + TP) // period) * period
    assert B == 1 and E == LANES and M == 8 and H == 32 and D % LANES == 0 and FF % LANES == 0
    assert SEG % 16 == 0 and S % (SEG * PASSES_PER_STEP) == 0 and 0 < TP <= SEG and TP % 8 == 0
    assert (RING - T0) % SEG == 0 and T0 % 128 == 0
    assert (S - T0) % (16 * KT) == 0

    hbm = pl.BlockSpec(memory_space=pl.ANY)
    scratch = [
        pltpu.VMEM((S, D), A_x.dtype),
        pltpu.VMEM((S, D), F32),
        pltpu.VMEM((KT, T0 // 2, LANES), U32),
        pltpu.VMEM((S, D), A_x.dtype),
        *[pltpu.VMEM((H, D // 2, E), U32)] * 3,
        pltpu.VMEM((KT, H * E, LANES), BF16),
        *[pltpu.VMEM((LANES * H, E), BF16)] * 3,
        *[pltpu.VMEM((FF // LANES, D, LANES), BF16)] * 2,
        pltpu.VMEM((KT, FF, LANES), BF16),
        pltpu.VMEM((M, D), A_mem0.dtype),
        pltpu.VMEM((M, D), F32),
        pltpu.VMEM((M + SEG, H * E), F32),
        pltpu.VMEM((M + SEG, D), F32),
        pltpu.VMEM((8, D), F32),
        pltpu.VMEM((2, 8, LANES), F32),
        pltpu.VMEM((2, 8, LANES), I32),
        pltpu.SemaphoreType.DMA((13,)),
        *[pltpu.VMEM((3, RING, E), F32)] * H,
        pltpu.VMEM((D,), B_w_r.dtype),
    ]
    out = pl.pallas_call(
        functools.partial(_kernel, S=S, D=D, H=H, E=E, M=M, SEG=SEG, FF=FF, TP=TP, T0=T0, RING=RING),
        out_shape=jax.ShapeDtypeStruct((S, D), A_x.dtype),
        in_specs=[hbm] * 10,
        out_specs=hbm,
        scratch_shapes=scratch,
        compiler_params=pltpu.CompilerParams(vmem_limit_bytes=120 * 1024 * 1024),
        name="rmt_mod",
    )(A_x.reshape(S, D), A_mem0.reshape(M, D),
      A_Wq.reshape(D * H, E), A_Wk.reshape(D * H, E), A_Wv.reshape(D * H, E),
      A_Wo.reshape(H * E, D), B_w_r, B_w_gate, B_w_up, B_w_down)
    return out.reshape(B, S, D)
```
